```python
import jax
import jax.numpy as jnp

def _softmax(x, axis=-1):
    return jax.nn.softmax(x, axis=axis)

def _gelu(x):
    return jax.nn.gelu(x, approximate=True)

def _silu(x):
    return jax.nn.silu(x)

def _sigmoid(x):
    return jax.nn.sigmoid(x)

def _layernorm(x, axis=-1, eps=1e-05):
    m = jnp.mean(x, axis=axis, keepdims=True)
    v = jnp.var(x, axis=axis, keepdims=True)
    return (x - m) / jnp.sqrt(v + eps)

def _scatter_add(tgt, idx, src, axis=0):
    return tgt.at[idx].add(src)

def _segment_sum(src, seg, n):
    return jax.ops.segment_sum(src, seg, n)

class _Rng:

    def __init__(self, key):
        self._k = key

    def _next(self):
        self._k, sub = jax.random.split(self._k)
        return sub

    def normal(self, shape):
        return jax.random.normal(self._next(), shape, dtype=jnp.bfloat16)

    def randint(self, lo, hi, shape):
        return jax.random.randint(self._next(), shape, lo, hi, dtype=jnp.int32)

    def uniform(self, shape, lo=0.0, hi=1.0):
        return jax.random.uniform(self._next(), shape, jnp.bfloat16, lo, hi)

    def permutation(self, n):
        return jax.random.permutation(self._next(), n)
kernel_name = 'interleave_layers__memory_aug_infini_attn__sliding_local_dilated__prompt'

def setup_inputs():
    _rng = _Rng(jax.random.key(int.from_bytes(__import__("os").urandom(4), "little")))
    _w = lambda a: (lambda t: t.astype(jnp.bfloat16) if jnp.issubdtype(t.dtype, jnp.floating) else t)(jnp.asarray(a))

    def _A_setup():
        B, S, D, H = (1, 2048, 1024, 32)
        N = 4
        L = max(1, S // N)
        sc = D ** (-0.5)
        return {'x': _w((lambda *s: _rng.normal(s) * 0.05)(B, N * L, D)), 'wq': _w((lambda *s: _rng.normal(s) * 0.05)(D, D) * sc), 'wk': _w((lambda *s: _rng.normal(s) * 0.05)(D, D) * sc), 'wv': _w((lambda *s: _rng.normal(s) * 0.05)(D, D) * sc), 'wo': _w((lambda *s: _rng.normal(s) * 0.05)(D, D) * sc), 'beta': _w((lambda *s: _rng.normal(s) * 0.05)(H))}
    _A_in = _A_setup()

    def _B_setup():
        B, S, D = (1, 2048, 1024)
        return {'x': _w((lambda *s: _rng.normal(s) * 0.05)(B, S, D)), 'wqkv': _w((lambda *s: _rng.normal(s) * 0.05)(D, 3 * D)), 'wo': _w((lambda *s: _rng.normal(s) * 0.05)(D, D))}
    _B_in = _B_setup()
    return {'A_x': _A_in['x'], 'A_wq': _A_in['wq'], 'A_wk': _A_in['wk'], 'A_wv': _A_in['wv'], 'A_wo': _A_in['wo'], 'A_beta': _A_in['beta'], 'B_x': _B_in['x'], 'B_wqkv': _B_in['wqkv'], 'B_wo': _B_in['wo']}

def reference(A_x, A_wq, A_wk, A_wv, A_wo, A_beta, B_x, B_wqkv, B_wo):

    def _A_ref(x, wq, wk, wv, wo, beta):
        B, S, D = x.shape
        H = 32
        Dh = D // H
        N = 4
        L = S // N
        q = (lambda x, *d: x.transpose(*d))((x @ wq).reshape(B, S, H, Dh), 0, 2, 1, 3).reshape(B, H, N, L, Dh)
        k = (lambda x, *d: x.transpose(*d))((x @ wk).reshape(B, S, H, Dh), 0, 2, 1, 3).reshape(B, H, N, L, Dh)
        v = (lambda x, *d: x.transpose(*d))((x @ wv).reshape(B, S, H, Dh), 0, 2, 1, 3).reshape(B, H, N, L, Dh)
        phi = lambda t: jnp.where(t > 0, t + 1.0, jnp.exp(t))
        scale = Dh ** (-0.5)
        ar = jnp.arange(L)
        mask = (lambda x, dt: x.astype(dt))(ar[:, None] < ar[None, :], x.dtype) * -1000000000.0
        g = _sigmoid(beta).reshape(1, H, 1, 1)
        M = jnp.einsum('bhd,bhe->bhde', q[:, :, 0, 0, :] * 0.0, q[:, :, 0, 0, :] * 0.0)
        z = q[:, :, 0, 0, :] * 0.0
        outs = []
        for s in range(N):
            qs, ks, vs = (q[:, :, s].copy(), k[:, :, s].copy(), v[:, :, s].copy())
            logits = jnp.einsum('bhqd,bhkd->bhqk', qs, ks) * scale + mask
            p = _softmax(logits, axis=-1)
            a_dot = jnp.einsum('bhqk,bhkd->bhqd', p, vs)
            pq = phi(qs)
            num = jnp.einsum('bhld,bhde->bhle', pq, M)
            den = jnp.einsum('bhld,bhd->bhl', pq, z)[..., None] + 1e-06
            a_mem = num / den
            o = g * a_mem + (1.0 - g) * a_dot
            outs.append(o)
            pk = phi(ks)
            M = M + jnp.einsum('bhld,bhle->bhde', pk, vs)
            z = z + jnp.einsum('bhld->bhd', pk)
        o = (lambda x, *d: x.transpose(*d))(jnp.stack(outs, 2).reshape(B, H, S, Dh), 0, 2, 1, 3).reshape(B, S, D)
        return o @ wo

    def _B_ref(x, wqkv, wo):
        B, S, D = x.shape
        H = 32
        Dh = D // H
        W, dil = (8, 2)
        qkv = (lambda x, *d: x.transpose(*d))((x @ wqkv).reshape(B, S, 3, H, Dh), 2, 0, 3, 1, 4)
        q, k, v = (qkv[0], qkv[1], qkv[2])
        scale = Dh ** (-0.5)
        pos = jnp.arange(S)
        off = jnp.arange(W) * dil
        idx = pos[:, None] - off[None, :]
        mask = idx >= 0
        idx_c = jnp.where(mask, idx, 0).reshape(-1)
        kg = k[:, :, idx_c, :].reshape(B, H, S, W, Dh)
        vg = v[:, :, idx_c, :].reshape(B, H, S, W, Dh)
        logits = jnp.einsum('bhsd,bhswd->bhsw', q, kg) * scale
        logits = jnp.where(mask[None, None, :, :], logits, -1000000000.0)
        attn = _softmax(logits, axis=-1)
        o = jnp.einsum('bhsw,bhswd->bhsd', attn, vg)
        return (lambda x, *d: x.transpose(*d))(o, 0, 2, 1, 3).reshape(B, S, D) @ wo
    x = A_x
    x = x + _A_ref(_layernorm(x, axis=-1), A_wq, A_wk, A_wv, A_wo, A_beta)
    x = x + _B_ref(_layernorm(x, axis=-1), B_wqkv, B_wo)
    x = x + _A_ref(_layernorm(x, axis=-1), A_wq, A_wk, A_wv, A_wo, A_beta)
    x = x + _B_ref(_layernorm(x, axis=-1), B_wqkv, B_wo)
    return x
```

```python
import functools
import math

import jax
import jax.numpy as jnp
from jax import lax
from jax.experimental import pallas as pl
from jax.experimental.pallas import tpu as pltpu

BF = jnp.bfloat16
F32 = jnp.float32
U32 = jnp.uint32
I32 = jnp.int32

S = 2048
D = 1024
H = 32
DH = 32
SEG = 512
NSEG = S // SEG
NG = D // 128
WIN = 8
DIL = 2
HALO = 16
NEG = -1e9
LOG2E = math.log2(math.e)
QSCALE = DH ** -0.5 * LOG2E

NT = (((1,), (1,)), ((), ()))


def _dot(a, b):
    return jnp.dot(a, b, preferred_element_type=F32)


def _phi(t):
    return jnp.where(t > 0, t + 1.0, jnp.exp(t))


def _layernorm(x):
    m = jnp.mean(x, axis=-1, keepdims=True)
    c = x - m
    v = jnp.mean(c * c, axis=-1, keepdims=True)
    return c * lax.rsqrt(v + 1e-5)


def _recip(x):
    r = pltpu.reciprocal(x, approx=True)
    return r * (2.0 - x * r)


def make(cfg=None):
    cfg = dict(cfg or {})
    TB = cfg.get("TB", 256)
    GU = cfg.get("GU", 4)
    RB = cfg.get("RB", 32)
    JORD = cfg.get("JORD", (3, 0, 2, 1))
    DEPTH = cfg.get("DEPTH", 2)
    NSLOT = 4
    NB = S // TB

    def kernel(x_hbm, wq_hbm, wk_hbm, wv_hbm, wo_hbm, beta_ref, wqkv_hbm, wob_hbm, out_hbm,
               xio, xres, xn, wq_st, wv_st, wk, wo, wqkv_st, wob_st, wqvT_u, wqkv_u, wob, wob_tmp,
               qT, pqT, vT, kk, pk, o_u, mem, gate, bias,
               qb, kb, vb, ob, sems, *sbufs):
        wqvT = wqvT_u.bitcast(BF)
        wqkv = wqkv_u.bitcast(BF)
        oa = o_u.bitcast(BF)

        def x_copy(s):
            return pltpu.make_async_copy(x_hbm.at[pl.ds(s * SEG, SEG)], xio.at[pl.ds(s * SEG, SEG)], sems.at[s])

        w_copies = [pltpu.make_async_copy(src, dst, sems.at[NSEG + i]) for i, (src, dst) in enumerate(
            [(wq_hbm, wq_st), (wv_hbm, wv_st), (wk_hbm, wk), (wo_hbm, wo), (wqkv_hbm, wqkv_st), (wob_hbm, wob_st)])]

        def out_copy(c):
            rows = pl.ds(pl.multiple_of(c * TB, TB), TB)
            return pltpu.make_async_copy(xio.at[rows], out_hbm.at[rows], sems.at[NSEG + 6 + c])

        x_copy(0).start()
        w_copies[0].start()
        w_copies[1].start()
        w_copies[2].start()

        ki = lax.broadcasted_iota(I32, (128, 128), 0)
        qi = lax.broadcasted_iota(I32, (128, 128), 1)
        bias[...] = jnp.where(ki <= qi, 0.0, NEG * LOG2E)
        b_row = jnp.broadcast_to(beta_ref[...].astype(F32), (H, H))
        diag = lax.broadcasted_iota(I32, (H, H), 0) == lax.broadcasted_iota(I32, (H, H), 1)
        b_col = jnp.sum(jnp.where(diag, b_row, 0.0), axis=1, keepdims=True)
        g_all = jax.nn.sigmoid(jnp.broadcast_to(b_col, (H, 128)))
        for h in range(H):
            gate[h] = jnp.broadcast_to(g_all[h:h + 1], (8, 128))

        x_copy(0).wait()
        for s in range(1, NSEG):
            x_copy(s).start()
        for r in range(0, SEG, 64):
            x0 = xio[r:r + 64, :].astype(F32)
            xres[r:r + 64, :] = x0
            xn[0, r:r + 64, :] = _layernorm(x0).astype(BF)
        w_copies[0].wait()
        w_copies[3].start()
        w_copies[4].start()
        w_copies[5].start()
        for g in range(0, NG, 2):
            t = wq_st[:, 128 * g:128 * g + 256].T
            wqvT[256 * g:256 * g + 128, :] = t[0:128]
            wqvT[256 * g + 256:256 * g + 384, :] = t[128:256]
        w_copies[1].wait()
        for g in range(0, NG, 2):
            t = wv_st[:, 128 * g:128 * g + 256].T
            wqvT[256 * g + 128:256 * g + 256, :] = t[0:128]
            wqvT[256 * g + 384:256 * g + 512, :] = t[128:256]
        w_copies[2].wait()
        for s in range(1, NSEG):
            x_copy(s).wait()

        def widen(s, c):
            rows = pl.ds(pl.multiple_of(s * 128, 128), 128)
            xres[rows, :] = xio[rows, :].astype(F32)
            return c
        lax.fori_loop(SEG // 128, S // 128, widen, 0)

        def prep_b_weights(s):
            lane = lax.broadcasted_iota(I32, (8, 128), 1)
            blk, sub = lane >> 4, lane & 15
            nrow = D // NSEG
            for r in range(0, nrow, 16):
                rows = pl.ds(pl.multiple_of(s * nrow + r, 16), 16)
                prow = pl.ds(pl.multiple_of((s * nrow + r) // 2, 8), 8)
                for part in range(3):
                    t = []
                    for g in range(NG):
                        w = pltpu.bitcast(wqkv_st[rows, part * D + 128 * g:part * D + 128 * g + 128], I32)
                        src = 32 * (sub & 3) + 4 * ((blk - g) & 7) + (sub >> 2)
                        t.append(jnp.take_along_axis(w, src, axis=1))
                    u = [t[(-j) % NG] for j in range(NG)]
                    for bit in (1, 2, 4):
                        m = (blk & bit) != 0
                        u = [jnp.where(m, u[(j - bit) % NG], u[j]) for j in range(NG)]
                    for j in range(NG):
                        src = 16 * ((((lane >> 2) & 7) + j) & 7) + 4 * (lane >> 5) + (lane & 3)
                        w = jnp.take_along_axis(u[j], src, axis=1)
                        wqkv_u[prow, part * D + 128 * j:part * D + 128 * j + 128] = pltpu.bitcast(w, U32)
            cols = pl.ds(pl.multiple_of(s * 256, 256), 256)
            for h in range(H):
                w = wob_st[32 * h:32 * h + 32, cols].astype(F32)
                wob_tmp[0, 33 * h:33 * h + 32, :] = w[:, 0:128]
                wob_tmp[1, 33 * h:33 * h + 32, :] = w[:, 128:256]
            for d in range(DH):
                w = jnp.concatenate([wob_tmp[i, pl.ds(d, H, stride=33), :] for i in range(2)], axis=1)
                wob[32 * d:32 * d + 32, cols] = w.astype(BF)

        def norm_rows(row0, n, slot, dst0):
            for r in range(0, n, 32):
                src = pl.ds(pl.multiple_of(row0 + r, 32), 32)
                dst = pl.ds(pl.multiple_of(dst0 + r, 32), 32)
                xn[slot, dst, :] = _layernorm(xres[src, :]).astype(BF)

        def scores(it, gg, j, sbuf, z):
            nk = 128 * (j + 1)
            cols = []
            for h in range(4):
                parts = [qT[it * GU + gg, 32 * h:32 * h + 32, 128 * j:128 * j + 128]]
                if h > 0:
                    parts.insert(0, jnp.zeros((32 * h, 128), BF))
                if h < 3:
                    parts.append(jnp.zeros((32 * (3 - h), 128), BF))
                cols.append(jnp.concatenate(parts, axis=0))
            s = _dot(kk[it, 0:nk, 128 * gg:128 * gg + 128], jnp.concatenate(cols, axis=1))
            mx = []
            for h in range(4):
                sh = s[:, 128 * h:128 * h + 128]
                sd = sh[nk - 128:] + bias[...]
                sh = sd if j == 0 else jnp.concatenate([sh[:nk - 128], sd], axis=0)
                sbuf[z, h, 0:nk, :] = sh
                mx.append(jnp.max(sh, axis=0, keepdims=True))
            return mx

        def memory(it, gg):
            g = it * GU + gg
            m = mem[g]
            rd = _dot(m.astype(BF), pqT[g])
            lhs = jnp.concatenate([vT[g], jnp.ones((16, SEG), BF)], axis=0)
            upd = _dot(lhs, pk[it, :, 128 * gg:128 * gg + 128])
            row = lax.broadcasted_iota(I32, (144, 128), 0)
            col = lax.broadcasted_iota(I32, (144, 128), 1) >> 5
            keep = jnp.where(row < 128, row >> 5, row - 128) == col
            mem[g] = m + jnp.where(keep, upd, 0.0)
            return rd

        def attend(it, gg, j, sbuf, z, mx, rd):
            nk = 128 * (j + 1)
            g = it * GU + gg
            inv_den = _recip(rd[128:136, 128 * j:128 * j + 128] + 1e-6)
            outs = []
            for h in range(4):
                p = jnp.exp2(sbuf[z, h, 0:nk, :] - mx[h])
                lhs = jnp.concatenate([vT[g, 32 * h:32 * h + 32, 0:nk], jnp.ones((16, nk), BF)], axis=0)
                r = _dot(lhs, p.astype(BF))
                gt = gate[4 * g + h]
                c_dot = (1.0 - gt) * _recip(r[32:40])
                c_mem = gt * jnp.broadcast_to(inv_den[h:h + 1], (8, 128))
                num = rd[32 * h:32 * h + 32, 128 * j:128 * j + 128]
                outs.append(r[0:32] * jnp.concatenate([c_dot] * 4, axis=0) + num * jnp.concatenate([c_mem] * 4, axis=0))
            oa[it, 128 * j:128 * j + 128, 128 * gg:128 * gg + 128] = jnp.concatenate(outs, axis=0).astype(BF).T

        def layer_a(l):
            mem[...] = jnp.zeros(mem.shape, F32)

            def seg_body(s, carry):
                slot = s & 1
                xs = xn[slot]
                for g in range(0, NG, 2):
                    qv = lax.dot_general(wqvT[256 * g:256 * g + 512, :], xs, NT, preferred_element_type=F32)
                    for i in range(2):
                        q = qv[256 * i:256 * i + 128]
                        qT[g + i] = (q * QSCALE).astype(BF)
                        pqT[g + i] = _phi(q).astype(BF)
                        vT[g + i] = qv[256 * i + 128:256 * i + 256].astype(BF)
                    k = _dot(xs, wk[:, 128 * g:128 * g + 256])
                    kk[g // GU, :, 128 * (g % GU):128 * (g % GU) + 256] = k.astype(BF)
                    pk[g // GU, :, 128 * (g % GU):128 * (g % GU) + 256] = _phi(k).astype(BF)
                norm_rows(((s + 1) & (NSEG - 1)) * SEG, SEG, 1 - slot, 0)

                def attn_body(it, c):
                    z0, z1 = it >> 10, it >> 11
                    items = [(gg, j) for gg in range(GU) for j in JORD]
                    mx, rd = {}, {}
                    for t in range(len(items) + DEPTH):
                        if t < len(items):
                            gg, j = items[t]
                            if gg not in rd:
                                rd[gg] = memory(it, gg)
                            mx[t] = scores(it, gg, j, sbufs[t % NSLOT], z0)
                        u = t - DEPTH
                        if u >= 0:
                            gg, j = items[u]
                            attend(it, gg, j, sbufs[u % NSLOT], z1, mx[u], rd[gg])
                    return c
                lax.fori_loop(0, NG // GU, attn_body, 0)

                @pl.when((l == 0) & (s == 0))
                def _():
                    w_copies[3].wait()
                    w_copies[4].wait()
                    w_copies[5].wait()

                rows = pl.ds(pl.multiple_of(s * SEG, SEG), SEG)
                o = jnp.concatenate([oa[i] for i in range(NG // GU)], axis=1)
                xres[rows, :] = xres[rows, :] + _dot(o, wo[...])
                prep_b_weights(s)
                return carry
            lax.fori_loop(0, NSEG, seg_body, 0)

        def layer_b(l):
            kb[:, 0:HALO, :] = jnp.zeros((NG, HALO, 128), F32)
            vb[:, 0:HALO, :] = jnp.zeros((NG, HALO, 128), F32)
            per_seg = SEG // TB

            def body(c, carry):
                z0, z1 = c >> 10, c >> 11
                seg = c // per_seg
                off = (c % per_seg) * TB
                slot = seg & 1
                xs = xn[slot, pl.ds(pl.multiple_of(off, TB), TB), :]
                for j in range(0, NG, 2):
                    q = _dot(xs, wqkv[:, 128 * j:128 * j + 256]) * QSCALE
                    k = _dot(xs, wqkv[:, D + 128 * j:D + 128 * j + 256])
                    for i in range(2):
                        qb[z0 + j + i] = q[:, 128 * i:128 * i + 128]
                        kb[z0 + j + i, HALO:HALO + TB, :] = k[:, 128 * i:128 * i + 128]
                for j in range(0, NG, 2):
                    v = _dot(xs, wqkv[:, 2 * D + 128 * j:2 * D + 128 * j + 256])
                    for i in range(2):
                        vb[z0 + j + i, HALO:HALO + TB, :] = v[:, 128 * i:128 * i + 128]
                norm_rows(((seg + 1) & (NSEG - 1)) * SEG + off, TB, 1 - slot, off)

                def taps(ref, j, r):
                    out = [None] * WIN
                    for a in range(WIN // 2):
                        slab = ref[z1 + j, pl.ds(HALO + r - 8 - DIL * a, RB + 8), :]
                        out[a] = slab[8:]
                        out[a + 4] = slab[:RB]
                    return out

                for r in range(0, TB, RB):
                    acc = [None] * WIN
                    for j in range(NG):
                        q = qb[z1 + j, r:r + RB, :]
                        for w, kt in enumerate(taps(kb, j, r)):
                            acc[w] = q * kt if j == 0 else acc[w] + q * kt
                    for w in range(WIN):
                        a = acc[w] + pltpu.roll(acc[w], 64, 1)
                        a = a + pltpu.roll(a, 32, 1)
                        if r < DIL * w:
                            pos = c * TB + r + lax.broadcasted_iota(I32, (RB, 128), 0)
                            a = jnp.where(pos >= DIL * w, a, NEG * LOG2E)
                        acc[w] = a
                    m = functools.reduce(jnp.maximum, acc)
                    p = [jnp.exp2(a - m) for a in acc]
                    inv = _recip(functools.reduce(lambda a, b: a + b, p))
                    p = [a * inv for a in p]
                    for j in range(0, NG, 2):
                        o2 = []
                        for i in range(2):
                            o = None
                            for w, vt in enumerate(taps(vb, j + i, r)):
                                o = p[w] * vt if o is None else o + p[w] * vt
                            o2.append(o)
                        ob[r:r + RB, 128 * j:128 * j + 256] = jnp.concatenate(o2, axis=1).astype(BF)
                for j in range(NG):
                    kb[z0 + j, 0:HALO, :] = kb[z1 + j, TB:TB + HALO, :]
                    vb[z0 + j, 0:HALO, :] = vb[z1 + j, TB:TB + HALO, :]

                rows = pl.ds(pl.multiple_of(c * TB, TB), TB)
                y = xres[rows, :] + _dot(ob[...], wob[...])
                xres[rows, :] = y
                xio[rows, :] = y.astype(BF)

                @pl.when(l == 1)
                def _():
                    out_copy(c).start()
                return carry
            lax.fori_loop(0, NB, body, 0)

        def pair(l, carry):
            layer_a(l)
            layer_b(l)
            return carry
        lax.fori_loop(0, 2, pair, 0)
        for c in range(NB):
            out_copy(c).wait()

    vm = pltpu.VMEM
    scratch = [
        vm((S, D), BF),
        vm((S, D), F32),
        vm((2, SEG, D), BF),
        vm((D, D), BF), vm((D, D), BF), vm((D, D), BF), vm((D, D), BF),
        vm((D, 3 * D), BF), vm((D, D), BF),
        vm((D, D), U32),
        vm((D // 2, 3 * D), U32),
        vm((D, D), BF),
        vm((2, 33 * H, 128), F32),
        vm((NG, 128, SEG), BF), vm((NG, 128, SEG), BF), vm((NG, 128, SEG), BF),
        vm((NG // GU, SEG, 128 * GU), BF), vm((NG // GU, SEG, 128 * GU), BF),
        vm((NG // GU, SEG // 2, 128 * GU), U32),
        vm((NG, 144, 128), F32),
        vm((H, 8, 128), F32),
        vm((128, 128), F32),
        vm((NG, TB, 128), F32), vm((NG, HALO + TB, 128), F32), vm((NG, HALO + TB, 128), F32),
        vm((TB, D), BF),
        pltpu.SemaphoreType.DMA((NSEG + 6 + NB,)),
    ] + [vm((1, 4, SEG, 128), F32)] * NSLOT

    hbm = pl.BlockSpec(memory_space=pl.ANY)

    def fn(A_x, A_wq, A_wk, A_wv, A_wo, A_beta, B_x, B_wqkv, B_wo):
        del B_x
        out = pl.pallas_call(
            kernel,
            out_shape=jax.ShapeDtypeStruct((S, D), BF),
            in_specs=[hbm, hbm, hbm, hbm, hbm, pl.BlockSpec(memory_space=pltpu.VMEM), hbm, hbm],
            out_specs=hbm,
            scratch_shapes=scratch,
            compiler_params=pltpu.CompilerParams(vmem_limit_bytes=110 * 2 ** 20, flags=cfg.get("flags")),
            name=cfg.get("name", "fused_layers"),
        )(A_x.reshape(S, D), A_wq, A_wk, A_wv, A_wo, A_beta.reshape(1, H), B_wqkv, B_wo)
        return out.reshape(A_x.shape)
    return fn


_fused = make()


@jax.jit
def pallas_interleave_layers__memory_aug_infini_attn__sliding_local_dilated__prompt_kernel(
    A_x: jax.Array,
    A_wq: jax.Array,
    A_wk: jax.Array,
    A_wv: jax.Array,
    A_wo: jax.Array,
    A_beta: jax.Array,
    B_x: jax.Array,
    B_wqkv: jax.Array,
    B_wo: jax.Array,
):
    return _fused(A_x, A_wq, A_wk, A_wv, A_wo, A_beta, B_x, B_wqkv, B_wo)
```

```python
import functools
import math

import jax
import jax.numpy as jnp
from jax import lax
from jax.experimental import pallas as pl
from jax.experimental.pallas import tpu as pltpu

BF = jnp.bfloat16
F32 = jnp.float32
U32 = jnp.uint32
I32 = jnp.int32

S = 2048
D = 1024
HD = D // 2
H = 32
DH = 32
SEG = 512
NSEG = S // SEG
NG = D // 128
NP = NG // 2
TB = 256
WIN = 8
DIL = 2
HALO = 16
NEG = -1e9
LOG2E = math.log2(math.e)
QSCALE = DH ** -0.5 * LOG2E

NT = (((1,), (1,)), ((), ()))


def _dot(a, b):
    return jnp.dot(a, b, preferred_element_type=F32)


def _phi(t):
    return jnp.where(t > 0, t + 1.0, jnp.exp(t))


def _recip(x):
    r = pltpu.reciprocal(x, approx=True)
    return r * (2.0 - x * r)


def _cat(xs, axis):
    return xs[0] if len(xs) == 1 else jnp.concatenate(xs, axis=axis)


def _tree(op, xs):
    while len(xs) > 1:
        xs = [op(xs[i], xs[i + 1]) for i in range(0, len(xs), 2)]
    return xs[0]


def _lhs7(a11, a12, a21, a22):
    return [a11 + a22, a21 + a22, a11, a22, a11 + a12, a21 - a11, a12 - a22]


def _rhs7(b11, b12, b21, b22):
    return [b11 + b22, b11, b12 - b22, b21 - b11, b22, b11 + b12, b21 + b22]


def _tile(j):
    o = 128 * ((j >> 1) + 2 * (j & 1))
    return slice(o, o + 128)


class _Pacer:
    def __init__(self, tmp, step):
        self.tmp = tmp
        self.z = [step >> (10 + i) for i in range(5)]
        self.plan, self.due = {}, {}
        self.pending, self.ready = [], []
        self.k = 0

    def spread(self, fn, n, first, last, slack):
        for i in range(n):
            t = first + i * (last - first) / max(n - 1, 1)
            self.plan.setdefault(int(t), []).append((fn, i, t - int(t), slack and int(t) + slack))

    def product(self, thunk):
        for fn, i, go, when in self.pending:
            done = fn(i, go)
            if when:
                self.due[when] = done
        self.pending = []
        if self.k in self.due:
            self.ready.append(self.due.pop(self.k))
        y = thunk()
        for fn, i, frac, when in self.plan.pop(self.k, []):
            r = 8 * int(frac * (y.shape[0] // 8))
            self.pending.append((fn, i, y[r:r + 8, -128:], when))
        self.k += 1
        return y

    def finish(self):
        assert not self.plan and not self.pending

    def combine7(self, prod, emit=None):
        z, tmp = self.z, self.tmp

        def run(i):
            return self.product(functools.partial(prod, i))
        m = run(2)
        view = (slice(0, m.shape[0]), slice(0, m.shape[1]))

        def put(i, v):
            for t in self.ready:
                tmp[i][z[1], 256:264, 0:128] = t.astype(F32)
            self.ready = []
            tmp[i][(z[0],) + view] = v

        def get(i, n):
            return tmp[i][(z[n],) + view]
        put(0, m)
        put(1, run(0))
        put(2, run(6))
        put(3, run(1))
        m5 = run(4)
        c12 = get(0, 1) + m5
        emit(0, 1, c12) if emit else put(5, c12)
        put(4, (get(1, 1) + get(2, 1)) - m5)
        c22 = ((get(1, 2) - get(3, 2)) + get(0, 2)) + run(5)
        emit(1, 1, c22) if emit else put(6, c22)
        m4 = run(3)
        c21, c11 = get(3, 1) + m4, get(4, 1) + m4
        if emit:
            emit(1, 0, c21)
            emit(0, 0, c11)
            return None
        return _cat([c11, get(5, 1)], 1), _cat([c21, get(6, 1)], 1)


def make(cfg=None):
    cfg = dict(cfg or {})
    RB = cfg.get("RB", 8)
    RV = cfg.get("RV", 8)
    LR = cfg.get("LR", 8)
    ORD = cfg.get("ORD", ((0, 3), (0, 0), (1, 3), (1, 0), (0, 2), (0, 1), (1, 2), (1, 1)))
    DEPTH = cfg.get("DEPTH", 2)
    NSLOT = 4

    def kernel(x_hbm, wq_hbm, wk_hbm, wv_hbm, wo_hbm, beta_ref, wqkv_hbm, wob_hbm, out_hbm,
               xio, xn, xc, mean, rstd, wq_st, wv_st, wk_st, wo_st, wqkv_st, wob_st,
               wqvT, wk, wo, wqkv, wob, wob_tmp,
               qT, pqT, vT, kk, pk, oa_u, mem, gate, bias, rdb, otb,
               kb0, kb1, vb0, vb1, pb0, pb1, ob0, ob1, sems, *rest):
        sbufs, tmp = rest[:NSLOT], rest[NSLOT:]
        oa = oa_u.bitcast(BF)
        kbs, vbs, pbs, obs = (kb0, kb1), (vb0, vb1), (pb0, pb1), (ob0, ob1)

        def segment(s):
            return xio.at[pl.ds(pl.multiple_of(s * SEG, SEG), SEG)]

        def x_copy(s):
            return pltpu.make_async_copy(x_hbm.at[pl.ds(s * SEG, SEG)], xio.at[pl.ds(s * SEG, SEG)], sems.at[s])

        w_copies = [pltpu.make_async_copy(src, dst, sems.at[NSEG + i]) for i, (src, dst) in enumerate(
            [(wq_hbm, wq_st), (wv_hbm, wv_st), (wk_hbm, wk_st), (wo_hbm, wo_st),
             (wqkv_hbm, wqkv_st.at[pl.ds(0, D)]), (wob_hbm, wob_st.at[pl.ds(0, D)])])]

        def out_copy(s):
            rows = pl.ds(pl.multiple_of(s * SEG, SEG), SEG)
            return pltpu.make_async_copy(xio.at[rows], out_hbm.at[rows], sems.at[NSEG + 6 + s])

        def norm_mean(z, s, i, go):
            if go is not None:
                mean[z[1], SEG:SEG + 8, :] = go
            rows = slice(i * LR, i * LR + LR)
            m = jnp.mean(segment(s)[rows, :].astype(F32), axis=-1, keepdims=True)
            mean[z[0], rows, :] = jnp.broadcast_to(m, (LR, 128))
            return mean[z[2], i * LR:i * LR + 8, :]

        def norm_var(z, s, i, go):
            if go is not None:
                mean[z[0], SEG:SEG + 8, :] = go
            rows = slice(i * LR, i * LR + LR)
            x = segment(s + z[0])[rows, :].astype(F32) - _cat([mean[z[1], rows, :]] * NG, 1)
            xc[z[0], rows, :] = x
            v = jnp.mean(x * x, axis=-1, keepdims=True)
            rstd[z[0], rows, :] = lax.rsqrt(jnp.broadcast_to(v, (LR, 128)) + 1e-5)
            return rstd[z[2], i * LR:i * LR + 8, :]

        def norm_store(z, i, go):
            if go is not None:
                rstd[z[0], SEG:SEG + 8, :] = go
            half, r = divmod(i * LR, 128)
            a1, a2 = [xc[z[1], o:o + LR, :] * _cat([rstd[z[1], o:o + LR, :]] * NG, 1)
                      for o in (256 * half + r, 256 * half + r + 128)]
            for n, a in enumerate(_lhs7(a1[:, :HD], a1[:, HD:], a2[:, :HD], a2[:, HD:])):
                xn[n, i * LR:i * LR + LR, :] = a.astype(BF)
            return xn[z[2], i * LR:i * LR + 8, 0:128]

        x_copy(0).start()
        w_copies[0].start()

        ki = lax.broadcasted_iota(I32, (128, 128), 0)
        qi = lax.broadcasted_iota(I32, (128, 128), 1)
        bias[...] = jnp.where(ki <= qi, 0.0, NEG * LOG2E)
        b_row = jnp.broadcast_to(beta_ref[...].astype(F32), (H, H))
        diag = lax.broadcasted_iota(I32, (H, H), 0) == lax.broadcasted_iota(I32, (H, H), 1)
        b_col = jnp.sum(jnp.where(diag, b_row, 0.0), axis=1, keepdims=True)
        g_all = jax.nn.sigmoid(jnp.broadcast_to(b_col, (H, 128)))
        for h in range(H):
            gate[h] = jnp.broadcast_to(g_all[h:h + 1], (8, 128))

        x_copy(0).wait()
        w_copies[1].start()

        def first_norm(i, c):
            r = (i >> 1) * 256 + (i & 1) * 64
            a = []
            for o in (0, 128):
                x = xio[pl.ds(pl.multiple_of(r + o, 64), 64), :].astype(F32)
                x = x - jnp.mean(x, axis=-1, keepdims=True)
                a.append(x * lax.rsqrt(jnp.mean(x * x, axis=-1, keepdims=True) + 1e-5))
            for n, v in enumerate(_lhs7(a[0][:, :HD], a[0][:, HD:], a[1][:, :HD], a[1][:, HD:])):
                xn[n, pl.ds(pl.multiple_of(i * 64, 64), 64), :] = v.astype(BF)
            return c
        lax.fori_loop(0, 4, first_norm, 0)

        def transposed_combos(st, off):
            def body(p, c):
                t = st[:, pl.ds(pl.multiple_of(p * 256, 256), 256)].T.astype(F32)
                for i, b in enumerate(_rhs7(t[:128, :HD], t[128:, :HD], t[:128, HD:], t[128:, HD:])):
                    wqvT[p, i, off:off + 128, :] = b.astype(BF)
                return c
            lax.fori_loop(0, NP, body, 0)

        def even_odd(w):
            return (_cat([w[:, 256 * p:256 * p + 128] for p in range(NP)], 1),
                    _cat([w[:, 256 * p + 128:256 * p + 256] for p in range(NP)], 1))

        w_copies[0].wait()
        w_copies[2].start()
        transposed_combos(wq_st, 0)
        w_copies[1].wait()
        for s in range(1, NSEG):
            x_copy(s).start()
        w_copies[3].start()
        w_copies[4].start()
        w_copies[5].start()
        transposed_combos(wv_st, 128)
        w_copies[2].wait()

        def wk_body(i, c):
            rows = pl.ds(pl.multiple_of(i * 32, 32), 32)
            t1 = wk_st[rows, :].astype(F32)
            t2 = wk_st[pl.ds(pl.multiple_of(HD + i * 32, 32), 32), :].astype(F32)
            for n, b in enumerate(_rhs7(*even_odd(t1), *even_odd(t2))):
                for e in range(2):
                    wk[e, n, rows, :] = b[:, 256 * e:256 * e + 256].astype(BF)
            return c
        lax.fori_loop(0, HD // 32, wk_body, 0)

        def late_setup():
            for s in range(1, NSEG):
                x_copy(s).wait()
            w_copies[3].wait()

            def wo_body(i, c):
                src = (i >> 2) * 256 + (i & 3) * 32
                t1 = wo_st[pl.ds(pl.multiple_of(src, 32), 32), :].astype(F32)
                t2 = wo_st[pl.ds(pl.multiple_of(src + 128, 32), 32), :].astype(F32)
                for n, b in enumerate(_rhs7(*even_odd(t1), *even_odd(t2))):
                    wo[n, pl.ds(pl.multiple_of(i * 32, 32), 32), :] = b.astype(BF)
                return c
            lax.fori_loop(0, HD // 32, wo_body, 0)
            w_copies[4].wait()
            w_copies[5].wait()

        def permuted(rows, part):
            lane = lax.broadcasted_iota(I32, (8, 128), 1)
            blk, sub = lane >> 4, lane & 15
            t = []
            for g in range(NG):
                w = pltpu.bitcast(wqkv_st[rows, part * D + 128 * g:part * D + 128 * g + 128], I32)
                src = 32 * (sub & 3) + 4 * ((blk - g) & 7) + (sub >> 2)
                t.append(jnp.take_along_axis(w, src, axis=1))
            u = [t[(-j) % NG] for j in range(NG)]
            for bit in (1, 2, 4):
                m = (blk & bit) != 0
                u = [jnp.where(m, u[(j - bit) % NG], u[j]) for j in range(NG)]
            out = []
            for j in range(NG):
                src = 16 * ((((lane >> 2) & 7) + j) & 7) + 4 * (lane >> 5) + (lane & 3)
                out.append(pltpu.bitcast(jnp.take_along_axis(u[j], src, axis=1), BF).astype(F32))
            return out

        def prep_qkv(z, s, i, go):
            wqkv_st[D:D + 8, 0:128] = go.astype(BF)
            r, part = divmod(i, 3)
            rows = pl.ds(pl.multiple_of(s * (HD // NSEG) + 16 * r, 16), 16)
            rows2 = pl.ds(pl.multiple_of(HD + s * (HD // NSEG) + 16 * r, 16), 16)
            t1, t2 = permuted(rows, part), permuted(rows2, part)
            for n, b in enumerate(_rhs7(_cat(t1[0::2], 1), _cat(t1[1::2], 1), _cat(t2[0::2], 1), _cat(t2[1::2], 1))):
                wqkv[part, n, rows, :] = b.astype(BF)
            return wqkv[z[2] + part, 0, rows, 0:128][0:8]

        def prep_wo_rows(z, s, i, go):
            wob_st[D:D + 8, 0:128] = go.astype(BF)
            cols = pl.ds(pl.multiple_of(s * 256, 256), 256)
            for h in range(4 * i, 4 * i + 4):
                w = wob_st[32 * h:32 * h + 32, cols].astype(F32)
                wob_tmp[z[0], 33 * h:33 * h + 32, :] = w[:, 0:128]
                wob_tmp[z[0] + 1, 33 * h:33 * h + 32, :] = w[:, 128:256]
            return wob_tmp[z[2], 0:8, :]

        def prep_wo(z, s, d, go):
            wob_tmp[z[0], 33 * H:33 * H + 8, :] = go
            blocks = [wob_tmp[z[1] + i, pl.ds(dd, H, stride=33), :] for dd in (d, d + DH // 2) for i in range(2)]
            for n, b in enumerate(_rhs7(*blocks)):
                wob[s, n, 32 * d:32 * d + 32, :] = b.astype(BF)
            return wob[z[2] + s, 0, 0:8, :]

        def project(pc, it, e):
            p = 2 * it + e

            def prod_qv(i):
                return lax.dot_general(wqvT[p, i], xn[i], NT, preferred_element_type=F32)

            def emit_qv(half, o, c):
                q, lanes, g = c[:128], slice(256 * half, 256 * half + 256), pc.z[0] + 2 * e + o
                qT[g, :, lanes] = (q * QSCALE).astype(BF)
                pqT[g, :, lanes] = _phi(q).astype(BF)
                vT[g, :, lanes] = c[128:].astype(BF)
            ks = pc.combine7(lambda i: _dot(xn[i], wk[it, i, :, 128 * e:128 * e + 128]))
            for k, r0 in zip(ks, (0, 128)):
                for i in range(2):
                    rows = slice(256 * i + r0, 256 * i + r0 + 128)
                    kk[pc.z[0] + e, rows, :] = k[128 * i:128 * i + 128].astype(BF)
                    pk[pc.z[0] + e, rows, :] = _phi(k[128 * i:128 * i + 128]).astype(BF)
            pc.combine7(prod_qv, emit_qv)

        def lanes_of(g):
            return slice(128 * (g & 1), 128 * (g & 1) + 128)

        def scores(z, g, j, sbuf):
            nk = 128 * (j + 1)
            cols = []
            for h in range(4):
                parts = [qT[z[1] + g, 32 * h:32 * h + 32, _tile(j)]]
                if h > 0:
                    parts.insert(0, jnp.zeros((32 * h, 128), BF))
                if h < 3:
                    parts.append(jnp.zeros((32 * (3 - h), 128), BF))
                cols.append(_cat(parts, 0))
            s = _dot(kk[z[1] + g // 2, 0:nk, lanes_of(g)], _cat(cols, 1))
            mx = []
            for h in range(4):
                sh = s[:, 128 * h:128 * h + 128]
                sd = sh[nk - 128:] + bias[...]
                sh = sd if j == 0 else _cat([sh[:nk - 128], sd], 0)
                sbuf[z[0], h, 0:nk, :] = sh
                mx.append(jnp.max(sh, axis=0, keepdims=True))
            return mx

        def memory_read(z, it, g):
            rdb[z[0] + g] = _dot(mem[4 * it + g].astype(BF), pqT[z[1] + g])

        def memory_update(z, it, g):
            lhs = _cat([_cat([vT[z[1] + g, :, _tile(j)] for j in range(4)], 1), jnp.ones((16, SEG), BF)], 0)
            upd = _dot(lhs, pk[z[1] + g // 2, :, lanes_of(g)])
            row = lax.broadcasted_iota(I32, (144, 128), 0)
            col = lax.broadcasted_iota(I32, (144, 128), 1) >> 5
            keep = jnp.where(row < 128, row >> 5, row - 128) == col
            mem[4 * it + g] = mem[z[1] + 4 * it + g] + jnp.where(keep, upd, 0.0)

        def attend(z, it, g, j, sbuf, mx):
            nk = 128 * (j + 1)
            inv_den = _recip(rdb[z[1] + g, 128:136, _tile(j)] + 1e-6)
            outs = []
            for h in range(4):
                p = jnp.exp2(sbuf[z[1], h, 0:nk, :] - mx[h])
                vh = _cat([vT[z[1] + g, 32 * h:32 * h + 32, _tile(t)] for t in range(j + 1)], 1)
                r = _dot(_cat([vh, jnp.ones((16, nk), BF)], 0), p.astype(BF))
                gt = gate[16 * it + 4 * g + h]
                c_dot = (1.0 - gt) * _recip(r[32:40])
                c_mem = gt * jnp.broadcast_to(inv_den[h:h + 1], (8, 128))
                num = rdb[z[1] + g, 32 * h:32 * h + 32, _tile(j)]
                outs.append(r[0:32] * _cat([c_dot] * 4, 0) + num * _cat([c_mem] * 4, 0))
            return _cat(outs, 0)

        def add_residual(s, r0, n, ys):
            seg = segment(s)
            for y, o in zip(ys, (0, 128)):
                for i in range(y.shape[0] // 128):
                    view = (slice(r0 + 256 * i + o, r0 + 256 * i + o + 128), slice(256 * n, 256 * n + 256))
                    seg[view] = (seg[view].astype(F32) + y[128 * i:128 * i + 128]).astype(BF)

        def layer_a(l):
            mem[...] = jnp.zeros(mem.shape, F32)

            def heads_body(it, carry):
                pc = _Pacer(tmp, it)
                z = pc.z
                for e in range(2):
                    project(pc, it, e)
                items = [(2 * p + e, j) for p in range(2) for e, j in ORD]
                mx, o = {}, {}
                for g in range(4):
                    memory_read(z, it, g)
                for t in range(len(items) + DEPTH):
                    if t < len(items):
                        mx[t] = scores(z, *items[t], sbufs[t % NSLOT])
                    elif t - len(items) < 4:
                        memory_update(z, it, t - len(items))
                    u = t - DEPTH
                    if u >= 0:
                        g, j = items[u]
                        o[g, j] = attend(z, it, g, j, sbufs[u % NSLOT], mx[u])
                        g0, j0 = g & ~1, j & ~1
                        quad = [(g0, j0), (g0 + 1, j0), (g0, j0 + 1), (g0 + 1, j0 + 1)]
                        if all(k in o for k in quad):
                            tiles = [o[k] if k == (g, j) else otb[z[1] + k[0], :, _tile(k[1])] for k in quad]
                            for i, a in enumerate(_lhs7(*tiles)):
                                oa[it, i, 64 * j0:64 * j0 + 128, 64 * g0:64 * g0 + 128] = a.astype(BF).T
                        else:
                            otb[z[0] + g, :, _tile(j)] = o[g, j]
                for g in range(DEPTH, 4):
                    memory_update(z, it, g)
                return carry

            def seg_body(s, carry):
                lax.fori_loop(0, 2, heads_body, 0)

                @pl.when((l == 0) & (s == 0))
                def _():
                    late_setup()

                pc = _Pacer(tmp, s)
                z = pc.z
                nxt = (s + 1) & (NSEG - 1)
                for i in range(SEG // LR):
                    norm_mean(z, nxt, i, None)
                pc.spread(functools.partial(norm_var, z, nxt), SEG // LR, *cfg.get("AN1", (0, 5.9, 0)))
                pc.spread(functools.partial(norm_store, z), SEG // LR // 2, *cfg.get("AN2", (7, 25, 1)))
                if cfg.get("prep", True):
                    pc.spread(functools.partial(prep_qkv, z, s), 3 * HD // NSEG // 16, *cfg.get("AP0", (0, 23, 3)))
                    pc.spread(functools.partial(prep_wo_rows, z, s), H // 4, *cfg.get("AP1", (6, 13, 1)))
                    pc.spread(functools.partial(prep_wo, z, s), DH // 2, *cfg.get("AP2", (14, 25, 1)))
                for n in range(NP):
                    ys = pc.combine7(lambda i: _dot(_cat([oa[0, i], oa[1, i]], 1), wo[i, :, 128 * n:128 * n + 128]))
                    add_residual(s, 0, n, ys)
                pc.finish()
                return carry
            lax.fori_loop(0, NSEG, seg_body, 0)

        def layer_b(l):
            kb0[0:NG, 0:HALO, :] = jnp.zeros((NG, HALO, 128), F32)
            vb0[0:NG, 0:HALO, :] = jnp.zeros((NG, HALO, 128), F32)

            def body(s, carry):
                pc = _Pacer(tmp, s)
                z = pc.z

                def taps(ref, j, r, n):
                    out = [None] * WIN
                    for a in range(WIN // 2):
                        slab = ref[z[1] + j, pl.ds(HALO + r - 8 - DIL * a, n + 8), :]
                        out[a] = slab[8:]
                        out[a + 4] = slab[:n]
                    return out

                def probs(c, i, go):
                    kbs[c][z[0] + NG, 0:8, :] = go
                    r = (i >> 1) * RB + (i & 1) * 128
                    acc = [None] * WIN
                    for j in range(NG):
                        q = kbs[c][z[1] + NG + j, HALO + r:HALO + r + RB, :]
                        for w, kt in enumerate(taps(kbs[c], j, r, RB)):
                            acc[w] = q * kt if j == 0 else acc[w] + q * kt
                    acc = [a + pltpu.roll(a, 64, 1) for a in acc]
                    acc = [a + pltpu.roll(a, 32, 1) for a in acc]
                    for w in range(WIN):
                        if c == 0 and r < DIL * w:
                            pos = s * SEG + r + lax.broadcasted_iota(I32, (RB, 128), 0)
                            acc[w] = jnp.where(pos >= DIL * w, acc[w], NEG * LOG2E)
                    m = _tree(jnp.maximum, acc)
                    p = [jnp.exp2(a - m) for a in acc]
                    inv = _recip(_tree(jnp.add, p))
                    for w in range(WIN):
                        pbs[c][z[0] + w, r:r + RB, :] = p[w] * inv
                    return pbs[c][z[2], r:r + 8, :]

                def values(c, i, go):
                    vbs[c][z[0] + NG, 0:8, :] = go
                    r, e = (i >> 1) * RV, i & 1
                    a = []
                    for o in (r, r + 128):
                        p = [pbs[c][z[3 + e] + w, o:o + RV, :] for w in range(WIN)]
                        for j0 in (2 * e, 4 + 2 * e):
                            outs = []
                            for j in (j0, j0 + 1):
                                y = None
                                for w, vt in enumerate(taps(vbs[c], j, o, RV)):
                                    y = p[w] * vt if y is None else y + p[w] * vt
                                outs.append(y)
                            a.append(_cat(outs, 1))
                    for n, v in enumerate(_lhs7(*a)):
                        obs[c][z[0] + n, r:r + RV, 256 * e:256 * e + 256] = v.astype(BF)
                    return obs[c][z[2], r:r + 8, 256 * e:256 * e + 128]

                nxt = (s + 1) & (NSEG - 1)
                pc.spread(functools.partial(norm_mean, z, nxt), SEG // LR, *cfg.get("N0", (1, 20, 0)))
                pc.spread(functools.partial(norm_var, z, nxt), SEG // LR, *cfg.get("N1", (21, 53, 3)))
                pc.spread(functools.partial(probs, 0), TB // RB, *cfg.get("P0", (56, 100, 5)))
                pc.spread(functools.partial(values, 0), TB // RV, *cfg.get("V0", (105, 138, 2)))
                pc.spread(functools.partial(probs, 1), TB // RB, *cfg.get("P1", (140, 171, 5)))
                pc.spread(functools.partial(values, 1), TB // RV, *cfg.get("V1", (175, 192, 2)))
                pc.spread(functools.partial(norm_store, z), SEG // LR // 2, *cfg.get("N2", (194, 220, 2)))

                def project_b(c, part, p, refs, base):
                    def emit(half, e, y):
                        if part == 0:
                            y = y * QSCALE
                        refs[c][z[0] + base + 2 * p + e, HALO + 128 * half:HALO + 128 * half + 128, :] = y
                        if part > 0 and c == 0 and half == 1:
                            refs[1][z[0] + 2 * p + e, 0:HALO, :] = y[128 - HALO:]
                    pc.combine7(lambda i: _dot(xn[i, 128 * c:128 * c + 128, :], wqkv[part, i, :, 128 * p:128 * p + 128]), emit)

                for c in range(2):
                    for part, refs, base in ((0, kbs, NG), (1, kbs, 0), (2, vbs, 0)):
                        for p in range(NP):
                            project_b(c, part, p, refs, base)
                for c in range(2):
                    for n in range(NP):
                        add_residual(s, TB * c, n, pc.combine7(lambda i: _dot(obs[c][z[1] + i], wob[n, i])))
                pc.finish()
                for refs in (kbs, vbs):
                    for j in range(NG):
                        refs[0][z[0] + j, 0:HALO, :] = refs[1][z[2] + j, TB:TB + HALO, :]

                @pl.when(l == 1)
                def _():
                    out_copy(s).start()
                return carry
            lax.fori_loop(0, NSEG, body, 0)

        def pair(l, carry):
            if "A" in cfg.get("parts", "AB"):
                layer_a(l)
            if "B" in cfg.get("parts", "AB"):
                layer_b(l)
            return carry
        lax.fori_loop(0, 2, pair, 0)
        for s in range(NSEG):
            out_copy(s).wait()

    vm = pltpu.VMEM
    scratch = [
        vm((S, D), BF),
        vm((7, SEG // 2, HD), BF),
        vm((1, SEG, D), F32),
        vm((1, SEG + 8, 128), F32), vm((1, SEG + 8, 128), F32),
        vm((D, D), BF), vm((D, D), BF), vm((D, D), BF), vm((D, D), BF),
        vm((D + 16, 3 * D), BF), vm((D + 16, D), BF),
        vm((NP, 7, 256, HD), BF),
        vm((2, 7, HD, 256), BF), vm((7, HD, HD), BF),
        vm((3, 7, HD, HD), BF),
        vm((NP, 7, HD, 128), BF),
        vm((2, 33 * H + 8, 128), F32),
        vm((4, 128, SEG), BF), vm((4, 128, SEG), BF), vm((4, 128, SEG), BF),
        vm((2, SEG, 256), BF), vm((2, SEG, 256), BF),
        vm((2, 7, SEG // 4, 256), U32),
        vm((NG, 144, 128), F32),
        vm((H, 8, 128), F32),
        vm((128, 128), F32),
        vm((4, 144, SEG), F32),
        vm((4, 128, SEG), F32),
        *[vm((2 * NG, HALO + TB, 128), F32)] * 2,
        *[vm((NG + 1, HALO + TB, 128), F32)] * 2,
        *[vm((WIN, TB, 128), F32)] * 2,
        *[vm((7, TB // 2, HD), BF)] * 2,
        pltpu.SemaphoreType.DMA((2 * NSEG + 6,)),
    ] + [vm((1, 4, SEG, 128), F32)] * NSLOT + [vm((1, 264, 256), F32)] * 7

    hbm = pl.BlockSpec(memory_space=pl.ANY)

    def fn(A_x, A_wq, A_wk, A_wv, A_wo, A_beta, B_x, B_wqkv, B_wo):
        del B_x
        out = pl.pallas_call(
            kernel,
            out_shape=jax.ShapeDtypeStruct((S, D), BF),
            in_specs=[hbm, hbm, hbm, hbm, hbm, pl.BlockSpec(memory_space=pltpu.VMEM), hbm, hbm],
            out_specs=hbm,
            scratch_shapes=scratch,
            compiler_params=pltpu.CompilerParams(vmem_limit_bytes=110 * 2 ** 20, flags=cfg.get("flags")),
            name=cfg.get("name", "fused_layers"),
        )(A_x.reshape(S, D), A_wq, A_wk, A_wv, A_wo, A_beta.reshape(1, H), B_wqkv, B_wo)
        return out.reshape(A_x.shape)
    return fn


_fused = make()


@jax.jit
def pallas_interleave_layers__memory_aug_infini_attn__sliding_local_dilated__prompt_kernel(
    A_x: jax.Array,
    A_wq: jax.Array,
    A_wk: jax.Array,
    A_wv: jax.Array,
    A_wo: jax.Array,
    A_beta: jax.Array,
    B_x: jax.Array,
    B_wqkv: jax.Array,
    B_wo: jax.Array,
):
    return _fused(A_x, A_wq, A_wk, A_wv, A_wo, A_beta, B_x, B_wqkv, B_wo)
```

```python
import functools
import math

import jax
import jax.numpy as jnp
from jax import lax
from jax.experimental import pallas as pl
from jax.experimental.pallas import tpu as pltpu

BF = jnp.bfloat16
F32 = jnp.float32
U32 = jnp.uint32
I32 = jnp.int32

S = 2048
D = 1024
HD = D // 2
H = 32
DH = 32
SEG = 512
NSEG = S // SEG
NG = D // 128
NP = NG // 2
TB = 256
WIN = 8
DIL = 2
HALO = 16
NEG = -1e9
LOG2E = math.log2(math.e)
QSCALE = DH ** -0.5 * LOG2E

NT = (((1,), (1,)), ((), ()))


def _dot(a, b):
    return jnp.dot(a, b, preferred_element_type=F32)


def _phi(t):
    return jnp.where(t > 0, t + 1.0, jnp.exp(t))


def _recip(x):
    r = pltpu.reciprocal(x, approx=True)
    return r * (2.0 - x * r)


def _cat(xs, axis):
    return xs[0] if len(xs) == 1 else jnp.concatenate(xs, axis=axis)


def _tree(op, xs):
    while len(xs) > 1:
        xs = [op(xs[i], xs[i + 1]) for i in range(0, len(xs), 2)]
    return xs[0]


def _lhs7(a11, a12, a21, a22):
    return [a11 + a22, a21 + a22, a11, a22, a11 + a12, a21 - a11, a12 - a22]


LHS7 = ((0, 3, jnp.add), (2, 3, jnp.add), (0, 0, lambda a, b: a), (3, 3, lambda a, b: a),
        (0, 1, jnp.add), (2, 0, jnp.subtract), (1, 3, jnp.subtract))


def _rhs7(b11, b12, b21, b22):
    f11, f12, f21, f22 = [b.astype(F32) for b in (b11, b12, b21, b22)]
    return [b.astype(BF) for b in (f11 + f22, b11, f12 - f22, f21 - f11, b22, f11 + f12, f21 + f22)]


def _tile(j):
    o = 128 * j
    return slice(o, o + 128)


class _Pacer:
    def __init__(self, tmp, step):
        self.tmp = tmp
        self.z = [step >> (10 + i) for i in range(5)]
        self.plan, self.due = {}, {}
        self.pending, self.ready = [], []
        self.k = 0

    def spread(self, fn, n, first, last, slack):
        for i in range(n):
            t = first + i * (last - first) / max(n - 1, 1)
            self.plan.setdefault(int(t), []).append((fn, i, t - int(t), slack and t + slack))

    def product(self, thunk):
        for fn, i, go, when in self.pending:
            done = fn(i, go)
            if when and done is not None:
                self.due.setdefault(int(when), []).append((when - int(when), done))
        self.pending = []
        if self.k in self.due:
            self.ready += self.due.pop(self.k)
        y = thunk()
        for fn, i, frac, when in self.plan.pop(self.k, []):
            r = 8 * int(frac * (y.shape[0] // 8))
            self.pending.append((fn, i, y[r:r + 8, -128:], when))
        self.k += 1
        return y

    def after(self, t, x):
        bits = pltpu.bitcast(x, U32) | (pltpu.bitcast(t, U32) & self.z[0].astype(U32))
        return pltpu.bitcast(bits, x.dtype)

    def lhs(self, words):
        if self.ready:
            n = words.shape[0] // 8
            heads = [words[8 * i:8 * i + 8, 0:128] for i in range(n)]
            for frac, t in self.ready:
                heads[int(frac * n)] = self.after(t, heads[int(frac * n)])
            words = _cat([_cat(heads, 0), words[:, 128:]], 1)
            self.ready = []
        return pltpu.bitcast(words, BF)

    def finish(self):
        assert not self.plan and not self.pending

    def combine7(self, prod, emit=None):
        z, tmp = self.z, self.tmp

        def run(i):
            return self.product(functools.partial(prod, i))
        m = run(2)
        view = (slice(0, m.shape[0]), slice(0, m.shape[1]))

        def put(i, v):
            tmp[i][(z[0],) + view] = v

        def get(i, n):
            return tmp[i][(z[n],) + view]
        put(0, m)
        put(1, run(0))
        put(2, run(6))
        put(3, run(1))
        m5 = run(4)
        c12 = get(0, 1) + m5
        emit(0, 1, c12) if emit else put(5, c12)
        put(4, (get(1, 1) + get(2, 1)) - m5)
        c22 = ((get(1, 2) - get(3, 2)) + get(0, 2)) + run(5)
        emit(1, 1, c22) if emit else put(6, c22)
        m4 = run(3)
        c21, c11 = get(3, 1) + m4, get(4, 1) + m4
        if emit:
            emit(1, 0, c21)
            emit(0, 0, c11)
            return None
        return c11, get(5, 1), c21, get(6, 1)


def make(cfg=None):
    cfg = dict(cfg or {})
    RB = cfg.get("RB", 8)
    NW = cfg.get("NW", 128)
    LR = cfg.get("LR", 8)
    ORD = cfg.get("ORD", ((0, 3), (0, 2), (1, 3), (1, 2), (0, 1), (1, 1), (0, 0), (1, 0)))
    DEPTH = cfg.get("DEPTH", 2)
    NSLOT = 6
    PS = cfg.get('PS', 2)
    VSUM = cfg.get('VSUM', 64)
    CATCH = cfg.get('CATCH', 4)
    LAG = cfg.get('LAG', 2)
    VGO = cfg.get('VGO', True)
    import contextlib
    scope = jax.named_scope if cfg.get('prof') else (lambda n: contextlib.nullcontext())

    def scoped(name, f):
        def g(*a):
            with scope(name):
                return f(*a)
        return g

    def kernel(x_hbm, wq_hbm, wk_hbm, wv_hbm, wo_hbm, beta_ref, wqkv_hbm, wob_hbm, out_hbm,
               xio, xn_u, xc, mean, rstd, wq_st, wv_st, wo_st, wqkv_st, wob_st, perm0, perm1, perm2,
               wqvT_u, wk_u, wo_u, wqkv_u, wob_u, wob_tmp,
               oa_u, mem, gate, bias, rdb,
               kb0, kb1, vb0, vb1, pb0, pb1, ob0_u, ob1_u, sems, *rest):
        sbufs, tmp, otb, rest = rest[:NSLOT], rest[NSLOT:NSLOT + 7], rest[NSLOT + 7:NSLOT + 11], rest[NSLOT + 11:]
        qT, pqT, vT, kk, pk = [rest[2 * i:2 * i + 2] for i in range(5)]
        oa, xn, wqvT, wk, wo, wqkv, wob, ob0, ob1 = [
            r.bitcast(BF) for r in (oa_u, xn_u, wqvT_u, wk_u, wo_u, wqkv_u, wob_u, ob0_u, ob1_u)]
        wk_st = wqkv_st.at[0]
        kbs, vbs, pbs, obs = (kb0, kb1), (vb0, vb1), (pb0, pb1), (ob0, ob1)

        def segment(s):
            return xio.at[pl.ds(pl.multiple_of(s * SEG, SEG), SEG)]

        def x_copy(s):
            return pltpu.make_async_copy(x_hbm.at[pl.ds(s * SEG, SEG)], xio.at[pl.ds(s * SEG, SEG)], sems.at[s])

        w_copies = [pltpu.make_async_copy(src, dst, sems.at[NSEG + i]) for i, (src, dst) in enumerate(
            [(wq_hbm, wq_st), (wv_hbm, wv_st), (wk_hbm, wk_st), (wo_hbm, wo_st),
             *[(wqkv_hbm.at[:, pl.ds(D * i, D)], wqkv_st.at[i + 1]) for i in range(3)],
             (wob_hbm, wob_st.at[pl.ds(0, D)])])]

        def out_copy(s):
            rows = pl.ds(pl.multiple_of(s * SEG, SEG), SEG)
            return pltpu.make_async_copy(xio.at[rows], out_hbm.at[rows], sems.at[NSEG + 8 + s])

        def norm_mean(z, s, i, go):
            if go is not None:
                mean[z[1], SEG:SEG + 8, :] = go
            rows = slice(i * LR, i * LR + LR)
            m = jnp.mean(segment(s)[rows, :].astype(F32), axis=-1, keepdims=True)
            mean[z[0], rows, :] = jnp.broadcast_to(m, (LR, 128))
            return mean[z[2], i * LR:i * LR + 8, :]

        def norm_var(z, s, i, go):
            if go is not None:
                mean[z[0], SEG:SEG + 8, :] = go
            rows = slice(i * LR, i * LR + LR)
            x = segment(s + z[0])[rows, :].astype(F32) - _cat([mean[z[1], rows, :]] * NG, 1)
            xc[z[0], rows, :] = x
            v = jnp.mean(x * x, axis=-1, keepdims=True)
            rstd[z[0], rows, :] = lax.rsqrt(jnp.broadcast_to(v, (LR, 128)) + 1e-5)
            return rstd[z[2], i * LR:i * LR + 8, :]

        def norm_store(z, i, go):
            if go is not None:
                rstd[z[0], SEG:SEG + 8, :] = go
            i, e = divmod(i, HD // NW)
            half, r = divmod(i * 16, 128)
            a = [xc[z[1], o:o + 16, c:c + NW] * _cat([rstd[z[1], o:o + 16, :]] * (NW // 128), 1)
                 for o in (256 * half + r, 256 * half + r + 128) for c in (NW * e, HD + NW * e)]
            for n, v in enumerate(_lhs7(*a)):
                xn[n, i * 16:i * 16 + 16, NW * e:NW * e + NW] = v.astype(BF)
            return pltpu.bitcast(xn_u[z[2], i * 8:i * 8 + 8, NW * e:NW * e + 128], F32)

        x_copy(0).start()
        w_copies[0].start()

        ki = lax.broadcasted_iota(I32, (128, 128), 0)
        qi = lax.broadcasted_iota(I32, (128, 128), 1)
        bias[...] = jnp.where(ki <= qi, 0.0, NEG * LOG2E)
        b_row = jnp.broadcast_to(beta_ref[...].astype(F32), (H, H))
        diag = lax.broadcasted_iota(I32, (H, H), 0) == lax.broadcasted_iota(I32, (H, H), 1)
        b_col = jnp.sum(jnp.where(diag, b_row, 0.0), axis=1, keepdims=True)
        g_all = jax.nn.sigmoid(jnp.broadcast_to(b_col, (H, 128)))
        for h in range(H):
            gate[h] = jnp.broadcast_to(g_all[h:h + 1], (8, 128))

        x_copy(0).wait()
        w_copies[1].start()

        def first_norm(i, c):
            r = (i >> 1) * 256 + (i & 1) * 64
            a = []
            for o in (0, 128):
                x = xio[pl.ds(pl.multiple_of(r + o, 64), 64), :].astype(F32)
                x = x - jnp.mean(x, axis=-1, keepdims=True)
                a.append(x * lax.rsqrt(jnp.mean(x * x, axis=-1, keepdims=True) + 1e-5))
            for n, v in enumerate(_lhs7(a[0][:, :HD], a[0][:, HD:], a[1][:, :HD], a[1][:, HD:])):
                xn[n, pl.ds(pl.multiple_of(i * 64, 64), 64), :] = v.astype(BF)
            return c
        lax.fori_loop(0, 4, first_norm, 0)

        def transposed_combos(st, off):
            def body(p, c):
                t = st[:, pl.ds(pl.multiple_of(p * 256, 256), 256)].T.astype(F32)
                for i, b in enumerate(_rhs7(t[:128, :HD], t[128:, :HD], t[:128, HD:], t[128:, HD:])):
                    wqvT[p, i, off:off + 128, :] = b.astype(BF)
                return c
            lax.fori_loop(0, NP, body, 0)

        def even_odd(w):
            return (_cat([w[:, 256 * p:256 * p + 128] for p in range(NP)], 1),
                    _cat([w[:, 256 * p + 128:256 * p + 256] for p in range(NP)], 1))

        w_copies[0].wait()
        w_copies[2].start()
        transposed_combos(wq_st, 0)
        w_copies[1].wait()
        transposed_combos(wv_st, 128)
        w_copies[2].wait()
        for s in range(1, NSEG):
            x_copy(s).start()
        for cp in w_copies[3:]:
            cp.start()

        def wk_body(i, c):
            rows = pl.ds(pl.multiple_of(i * 32, 32), 32)
            t1 = wk_st[rows, :].astype(F32)
            t2 = wk_st[pl.ds(pl.multiple_of(HD + i * 32, 32), 32), :].astype(F32)
            for n, b in enumerate(_rhs7(*even_odd(t1), *even_odd(t2))):
                for e in range(2):
                    wk[e, n, rows, :] = b[:, 256 * e:256 * e + 256].astype(BF)
            return c
        lax.fori_loop(0, HD // 32, wk_body, 0)

        def late_setup():
            for s in range(1, NSEG):
                x_copy(s).wait()
            w_copies[3].wait()

            def wo_body(i, c):
                src = (i >> 2) * 256 + (i & 3) * 32
                t1 = wo_st[pl.ds(pl.multiple_of(src, 32), 32), :].astype(F32)
                t2 = wo_st[pl.ds(pl.multiple_of(src + 128, 32), 32), :].astype(F32)
                for n, b in enumerate(_rhs7(*even_odd(t1), *even_odd(t2))):
                    wo[n, pl.ds(pl.multiple_of(i * 32, 32), 32), :] = b.astype(BF)
                return c
            lax.fori_loop(0, HD // 32, wo_body, 0)
            for cp in w_copies[4:]:
                cp.wait()

        lane = lax.broadcasted_iota(I32, (8, 128), 1)

        def prep_spread(z, s, it, i, go):
            perm0[z[1], 256:264, :] = pltpu.bitcast(go, U32)
            g, k = divmod(i, 4)
            rows = pl.ds(pl.multiple_of(256 * it, 256) + (k >> 1) * HD + (k & 1) * 128, 128)
            w = pltpu.bitcast(wqkv_st[s, rows, 128 * g:128 * g + 128], U32)
            src = 32 * (lane & 3) + 4 * (((lane >> 4) - g) & 7) + ((lane & 15) >> 2)
            perm0[z[0] + g, 64 * k:64 * k + 64, :] = jnp.take_along_axis(w, _cat([src] * 8, 0), axis=1)
            return perm0[z[2] + g, 64 * k:64 * k + 8, :]

        def prep_exchange(z, i, go):
            perm0[z[0], 256:264, :] = pltpu.bitcast(go, U32)
            u = [perm0[z[1] + (-j) % NG, 8 * i:8 * i + 8, :] for j in range(NG)]
            for bit in (1, 2, 4):
                m = (lane & (16 * bit)) != 0
                u = [jnp.where(m, u[(j - bit) % NG], u[j]) for j in range(NG)]
            for j in range(NG):
                perm1[z[0] + j, 8 * i:8 * i + 8, :] = u[j]
            return perm1[z[2], 8 * i:8 * i + 8, :]

        def prep_collect(z, i, go):
            perm1[z[0], 256:264, :] = pltpu.bitcast(go, U32)
            j, k = divmod(i, 4)
            src = 16 * (((lane >> 2) + j) & 7) + 4 * (lane >> 5) + (lane & 3)
            w = perm1[z[1] + j, 64 * k:64 * k + 64, :]
            perm2[z[0] + j, 64 * k:64 * k + 64, :] = jnp.take_along_axis(w, _cat([src] * 8, 0), axis=1)
            return perm2[z[2] + j, 64 * k:64 * k + 8, :]

        def prep_combine(z, s, it, i, go):
            perm2[z[0], 256:264, :] = pltpu.bitcast(go, U32)
            r, p = divmod(i, NP)
            w = [pltpu.bitcast(perm2[z[1] + 2 * p + e, o + 8 * r:o + 8 * r + 8, :], BF) for o in (0, 128) for e in range(2)]
            rows = pl.ds(pl.multiple_of(256 * it, 256) + 16 * r, 16)
            for n, b in enumerate(_rhs7(*w)):
                wqkv[s, n, rows, 128 * p:128 * p + 128] = b
            return pltpu.bitcast(wqkv[z[2] + s, 0, rows, 128 * p:128 * p + 128], U32)

        def prep_wo_rows(z, s, i, go):
            wob_st[D:D + 8, 0:128] = go.astype(BF)
            cols = pl.ds(pl.multiple_of(s * 256, 256), 256)
            for h in range(i, i + 1):
                w = wob_st[32 * h:32 * h + 32, cols].astype(F32)
                wob_tmp[z[0], 33 * h:33 * h + 32, :] = w[:, 0:128]
                wob_tmp[z[0] + 1, 33 * h:33 * h + 32, :] = w[:, 128:256]
            return wob_tmp[z[2], 0:8, :]

        def prep_wo(z, s, i, go):
            wob_tmp[z[0], 33 * H:33 * H + 8, :] = go
            d, e = divmod(i, 2)
            blocks = [wob_tmp[z[1] + c, pl.ds(33 * 16 * e + dd, 16, stride=33), :] for dd in (d, d + DH // 2) for c in range(2)]
            for n, b in enumerate(_rhs7(*blocks)):
                wob[n, 16 * i:16 * i + 16, pl.ds(pl.multiple_of(s * 128, 128), 128)] = b.astype(BF)
            return pltpu.bitcast(wob_u[z[2], 0:8, pl.ds(pl.multiple_of(s * 128, 128), 128)], F32)

        def project(pc, it, e):
            z = pc.z
            c11, c12, c21, c22 = pc.combine7(lambda i: _dot(pc.lhs(xn_u[i]), wk[it, i, :, 128 * e:128 * e + 128]))
            for k, r0 in ((_cat([c11, c12], 1), 0), (_cat([c21, c22], 1), 128)):
                for i in range(2):
                    rows = slice(256 * i + r0, 256 * i + r0 + 128)
                    kk[e][z[0], rows, :] = k[128 * i:128 * i + 128].astype(BF)
                    pk[e][z[0], rows, :] = _phi(k[128 * i:128 * i + 128]).astype(BF)
            for c in range(2):
                c11, c12, c21, c22 = pc.combine7(lambda i: lax.dot_general(
                    pc.lhs(wqvT_u[z[c] + 2 * it + e, i]), xn[i, 128 * c:128 * c + 128, :], NT, preferred_element_type=F32))
                for o, y in enumerate((_cat([c11, c21], 1), _cat([c12, c22], 1))):
                    q, lanes, g = y[:128], slice(256 * c, 256 * c + 256), z[0] + o
                    qT[e][g, :, lanes] = (q * QSCALE).astype(BF)
                    pqT[e][g, :, lanes] = _phi(q).astype(BF)
                    vT[e][g, :, lanes] = y[128:].astype(BF)

        def lanes_of(g):
            return slice(128 * (g & 1), 128 * (g & 1) + 128)

        def scores(z, g, j, t, sbuf, mx):
            cols = []
            for h in range(4):
                parts = [qT[g // 2][z[1 + t] + g % 2, 32 * h:32 * h + 32, _tile(j)]]
                if h > 0:
                    parts.insert(0, jnp.zeros((32 * h, 128), BF))
                if h < 3:
                    parts.append(jnp.zeros((32 * (3 - h), 128), BF))
                cols.append(_cat(parts, 0))
            s = _dot(kk[g // 2][z[1], _tile(t), lanes_of(g)], _cat(cols, 1))
            for h in range(4):
                sh = s[:, 128 * h:128 * h + 128]
                if t == j:
                    sh = sh + bias[...]
                sbuf[z[0], h, _tile(t), :] = sh
                for i in range(0, 128, 8):
                    mx[h] = sh[i:i + 8] if mx[h] is None else jnp.maximum(mx[h], sh[i:i + 8])
                if t == j:
                    mx[h] = jnp.max(mx[h], axis=0, keepdims=True)

        def memory_read(z, it, g):
            rdb[z[0] + g] = _dot(mem[4 * it + g].astype(BF), pqT[g // 2][z[1] + g % 2])

        def memory_update(z, it, g):
            lhs = _cat([_cat([vT[g // 2][z[1] + g % 2, :, _tile(j)] for j in range(4)], 1), jnp.ones((16, SEG), BF)], 0)
            upd = _dot(lhs, pk[g // 2][z[1], :, lanes_of(g)])
            head = lane >> 5
            keep = _cat([head == (r // 4) for r in range(16)] + [head == lax.broadcasted_iota(I32, (8, 128), 0)] * 2, 0)
            mem[4 * it + g] = mem[z[1] + 4 * it + g] + jnp.where(keep, upd, 0.0)

        def attend(pc, g, t, sbuf, mx, acc, tot):
            z = pc.z
            for h in range(4):
                p = jnp.exp2(sbuf[z[1], h, _tile(t), :] - mx[h])
                vh = vT[g // 2][z[1] + g % 2, 32 * h:32 * h + 32, _tile(t)]
                if VSUM:
                    parts = []
                    for i in range(128 - VSUM, -1, -VSUM):
                        part = _tree(jnp.add, [p[i + n:i + n + 8] for n in range(0, VSUM, 8)])
                        tot[h] = part if tot[h] is None else tot[h] + part
                        parts = [pc.after(tot[h], p[i:i + 8]), p[i + 8:i + VSUM]] + parts
                    r = _dot(vh, _cat(parts, 0).astype(BF))
                else:
                    r = _dot(_cat([vh, jnp.ones((16, 128), BF)], 0), p.astype(BF))[0:40]
                acc[h] = r if acc[h] is None else acc[h] + r

        def finish_tile(z, it, g, j, acc, tot):
            inv_den = _recip(rdb[z[1] + g, 128:136, _tile(j)] + 1e-6)
            outs = []
            for h in range(4):
                l = jnp.broadcast_to(jnp.sum(tot[h], axis=0, keepdims=True), (8, 128)) if VSUM else acc[h][32:40]
                gt = gate[16 * it + 4 * g + h]
                c_dot = (1.0 - gt) * _recip(l)
                c_mem = gt * jnp.broadcast_to(inv_den[h:h + 1], (8, 128))
                num = rdb[z[1] + g, 32 * h:32 * h + 32, _tile(j)]
                outs.append(acc[h][0:32] * _cat([c_dot] * 4, 0) + num * _cat([c_mem] * 4, 0))
            return _cat(outs, 0)

        def add_residual(s, r0, n, ys):
            seg = segment(s)
            for y, o in ((_cat(ys[:2], 1), 0), (_cat(ys[2:], 1), 128)):
                for i in range(y.shape[0] // 128):
                    view = (slice(r0 + 256 * i + o, r0 + 256 * i + o + 128), slice(256 * n, 256 * n + 256))
                    seg[view] = (seg[view].astype(F32) + y[128 * i:128 * i + 128]).astype(BF)

        def layer_a(l):
            mem[...] = jnp.zeros(mem.shape, F32)

            def heads_body(s, it, carry):
                pc = _Pacer(tmp, it)
                z = pc.z
                pc.spread(functools.partial(prep_spread, z, s, it), 32, *cfg.get("H0", (0, 8, 1.5)))
                pc.spread(functools.partial(prep_exchange, z), 32, *cfg.get("H1", (9, 16, 1.2)))
                pc.spread(functools.partial(prep_collect, z), 32, *cfg.get("H2", (17, 24, 1.5)))
                pc.spread(functools.partial(prep_combine, z, s, it), 64, *cfg.get("H3", (25, 39, 1.2)))
                for e in range(2):
                    project(pc, it, e)
                pc.finish()
                items = [(2 * p + e, j) for p in range(2) for e, j in ORD]
                units = [(n, g, j, t) for n, (g, j) in enumerate(items) for t in range(j + 1)]
                state = [([None] * 4, [None] * 4, [None] * 4) for _ in items]
                last = {n: k for k, (n, *_) in enumerate(units)}
                seen = set()

                def consume(n, g, j, t):
                    attend(pc, g, t, sbufs[n % NSLOT], *state[n])
                    if t < j:
                        return
                    o = finish_tile(z, it, g, j, *state[n][1:])
                    g0, j0, me = g & ~1, j & ~1, 2 * (j & 1) + (g & 1)
                    seen.add((g0, j0, me))
                    if sum((g0, j0, q) in seen for q in range(4)) < 4:
                        otb[me][z[0]] = o
                    for i, (x, y, op) in enumerate(LHS7):
                        if me in (x, y) and (g0, j0, x) in seen and (g0, j0, y) in seen:
                            a, b = [o if q == me else otb[q][z[1 + me]] for q in (x, y)]
                            oa[it, i, 64 * j0:64 * j0 + 128, 64 * g0:64 * g0 + 128] = op(a, b).astype(BF).T

                u, k, upd = 0, 0, 0
                while u < len(units):
                    if k < 4:
                        memory_read(z, it, k)
                    if k < len(units):
                        n, g, j, t = units[k]
                        scores(z, g, j, t, sbufs[n % NSLOT], state[n][0])
                    elif upd < 4:
                        memory_update(z, it, upd)
                        upd += 1
                    for _ in range(2 if k >= len(units) - CATCH else 1):
                        if u < len(units) and last[units[u][0]] + LAG <= k:
                            consume(*units[u])
                            u += 1
                    k += 1
                for g in range(upd, 4):
                    memory_update(z, it, g)
                return carry

            def seg_body(s, carry):
                lax.fori_loop(0, 2, scoped('heads', functools.partial(heads_body, s)), 0)

                @pl.when((l == 0) & (s == 0))
                def _():
                    scoped('late', late_setup)()

                pc = _Pacer(tmp, s)
                z = pc.z
                nxt = (s + 1) & (NSEG - 1)
                for i in range(SEG // LR):
                    norm_mean(z, nxt, i, None)
                pc.spread(functools.partial(norm_var, z, nxt), SEG // LR, *cfg.get("AN1", (0, 5.9, 0)))
                pc.spread(functools.partial(norm_store, z), SEG // 32 * (HD // NW), *cfg.get("AN2", (7, 25.5, 1.2)))
                if cfg.get("prep", True):
                    pc.spread(functools.partial(prep_wo_rows, z, s), H, *cfg.get("AP1", (6, 13, 1.2)))
                    pc.spread(functools.partial(prep_wo, z, s), DH, *cfg.get("AP2", (14, 25.5, 1.2)))
                for n in range(NP):
                    ys = pc.combine7(lambda i: _dot(pc.lhs(_cat([oa_u[0, i], oa_u[1, i]], 1)), wo[i, :, 128 * n:128 * n + 128]))
                    add_residual(s, 0, n, ys)
                pc.finish()
                return carry
            lax.fori_loop(0, NSEG, scoped('segA', seg_body), 0)

        def layer_b(l):
            kb0[0:NG, 0:HALO, :] = jnp.zeros((NG, HALO, 128), F32)
            vb0[0:NG, 0:HALO, :] = jnp.zeros((NG, HALO, 128), F32)

            def body(s, carry):
                pc = _Pacer(tmp, s)
                z = pc.z

                def taps(ref, j, r, n):
                    out = [None] * WIN
                    for a in range(WIN // 2):
                        slab = ref[z[1] + j, pl.ds(HALO + r - 8 - DIL * a, n + 8), :]
                        out[a] = slab[8:]
                        out[a + 4] = slab[:n]
                    return out

                held = {}

                def probs(c, i, go):
                    kbs[c][z[0] + NG, 0:8, :] = go
                    i, step = divmod(i, PS)
                    r = (i >> 1) * RB + (i & 1) * 128
                    acc = held.pop(("k", c), [None] * WIN)
                    for j in range(step * NG // PS, (step + 1) * NG // PS):
                        q = kbs[c][z[1] + NG + j, HALO + r:HALO + r + RB, :]
                        for w, kt in enumerate(taps(kbs[c], j, r, RB)):
                            acc[w] = q * kt if j == 0 else acc[w] + q * kt
                    if step < PS - 1:
                        held["k", c] = acc
                        return None
                    acc = [a + pltpu.roll(a, 64, 1) for a in acc]
                    acc = [a + pltpu.roll(a, 32, 1) for a in acc]
                    for w in range(WIN):
                        if c == 0 and r < DIL * w:
                            pos = s * SEG + r + lax.broadcasted_iota(I32, (RB, 128), 0)
                            acc[w] = jnp.where(pos >= DIL * w, acc[w], NEG * LOG2E)
                    m = _tree(jnp.maximum, acc)
                    p = [jnp.exp2(a - m) for a in acc]
                    inv = _recip(_tree(jnp.add, p))
                    for w in range(WIN):
                        pbs[c][z[0] + w, r:r + RB, :] = p[w] * inv
                    return pbs[c][z[2], r:r + 8, :]

                def values(c, i, go):
                    i, step = divmod(i, 5)
                    r, e = 16 * (i // 4), i % 4
                    if step == 4:
                        for n, v in enumerate(_lhs7(*held.pop(("v", c)))):
                            obs[c][z[0] + n, r:r + 16, 128 * e:128 * e + 128] = v.astype(BF)
                        return pltpu.bitcast(obs[c][z[2], r:r + 16, 128 * e:128 * e + 128], F32)
                    if VGO:
                        vbs[c][z[0] + NG, 0:8, :] = go
                    o, j = r + 128 * (step >> 1), e + 4 * (step & 1)
                    y = None
                    for w, vt in enumerate(taps(vbs[c], j, o, 16)):
                        t = pbs[c][z[1 + e] + w, o:o + 16, :] * vt
                        y = t if y is None else y + t
                    held.setdefault(("v", c), []).append(y)
                    return pltpu.bitcast(y[0:8], U32) | pltpu.bitcast(y[8:16], U32)

                nxt = (s + 1) & (NSEG - 1)
                pc.spread(functools.partial(norm_mean, z, nxt), SEG // LR, *cfg.get("N0", (1, 20, 0)))
                pc.spread(functools.partial(norm_var, z, nxt), SEG // LR, *cfg.get("N1", (21, 53, 4)))
                pc.spread(functools.partial(probs, 0), PS * TB // RB, *cfg.get("P0", (56, 106, 6)))
                pc.spread(functools.partial(values, 0), 5 * TB // 8, *cfg.get("V0", (144, 165.5, 2)))
                pc.spread(functools.partial(probs, 1), PS * TB // RB, *cfg.get("P1", (112, 146, 5.5)))
                pc.spread(functools.partial(values, 1), 5 * TB // 8, *cfg.get("V1", (168, 193.5, 2)))
                pc.spread(functools.partial(norm_store, z), SEG // 32 * (HD // NW), *cfg.get("N2", (194, 220, 2.5)))

                def project_b(c, part, p, refs, base):
                    def emit(half, e, y):
                        if part == 0:
                            y = y * QSCALE
                        refs[c][z[0] + base + 2 * p + e, HALO + 128 * half:HALO + 128 * half + 128, :] = y
                        if part > 0 and c == 0 and half == 1:
                            refs[1][z[0] + 2 * p + e, 0:HALO, :] = y[128 - HALO:]
                    pc.combine7(lambda i: _dot(pc.lhs(xn_u[i, 64 * c:64 * c + 64, :]), wqkv[part + 1, i, :, 128 * p:128 * p + 128]), emit)

                for c, part in cfg.get('BORD', ((0, 0), (0, 1), (1, 0), (1, 1), (0, 2), (1, 2))):
                    for p in range(NP):
                        project_b(c, part, p, (kbs, kbs, vbs)[part], NG if part == 0 else 0)
                for c in range(2):
                    for n in range(NP):
                        add_residual(s, TB * c, n, pc.combine7(lambda i: _dot(pc.lhs((ob0_u, ob1_u)[c][z[1 + n] + i]), wob[i, :, 128 * n:128 * n + 128])))
                pc.finish()
                for refs in (kbs, vbs):
                    for j in range(NG):
                        refs[0][z[0] + j, 0:HALO, :] = refs[1][z[2] + j, TB:TB + HALO, :]

                @pl.when(l == 1)
                def _():
                    out_copy(s).start()
                return carry
            lax.fori_loop(0, NSEG, scoped('segB', body), 0)

        def pair(l, carry):
            if "A" in cfg.get("parts", "AB"):
                layer_a(l)
            if "B" in cfg.get("parts", "AB"):
                layer_b(l)
            return carry
        lax.fori_loop(0, 2, scoped('pair', pair), 0)
        for s in range(NSEG):
            out_copy(s).wait()

    vm = pltpu.VMEM
    scratch = [
        vm((S, D), BF),
        vm((7, SEG // 4, HD), U32),
        vm((1, SEG, D), F32),
        vm((1, SEG + 8, 128), F32), vm((1, SEG + 8, 128), F32),
        vm((D, D), BF), vm((D, D), BF), vm((D, D), BF),
        vm((4, D, D), BF), vm((D + 16, D), BF), *[vm((NG, 264, 128), U32)] * 3,
        vm((NP, 7, 128, HD), U32),
        vm((2, 7, HD // 2, 256), U32), vm((7, HD // 2, HD), U32),
        vm((4, 7, HD // 2, HD), U32),
        vm((7, HD // 2, HD), U32),
        vm((2, 33 * H + 8, 128), F32),
        vm((2, 7, SEG // 4, 256), U32),
        vm((NG, 144, 128), F32),
        vm((H, 8, 128), F32),
        vm((128, 128), F32),
        vm((4, 144, SEG), F32),
        *[vm((2 * NG, HALO + TB, 128), F32)] * 2,
        *[vm((NG + 1, HALO + TB, 128), F32)] * 2,
        *[vm((WIN, TB, 128), F32)] * 2,
        *[vm((7, TB // 4, HD), U32)] * 2,
        pltpu.SemaphoreType.DMA((2 * NSEG + 8,)),
    ] + [vm((1, 4, SEG, 128), F32)] * NSLOT + [vm((1, 256, 128), F32)] * 7 + [vm((1, 128, 128), F32)] * 4 + [vm((2, 128, SEG), BF)] * 6 + [vm((1, SEG, 256), BF)] * 4

    hbm = pl.BlockSpec(memory_space=pl.ANY)

    def fn(A_x, A_wq, A_wk, A_wv, A_wo, A_beta, B_x, B_wqkv, B_wo):
        del B_x
        out = pl.pallas_call(
            kernel,
            out_shape=jax.ShapeDtypeStruct((S, D), BF),
            in_specs=[hbm, hbm, hbm, hbm, hbm, pl.BlockSpec(memory_space=pltpu.VMEM), hbm, hbm],
            out_specs=hbm,
            scratch_shapes=scratch,
            compiler_params=pltpu.CompilerParams(vmem_limit_bytes=110 * 2 ** 20, flags=cfg.get("flags")),
            name=cfg.get("name", "fused_layers"),
        )(A_x.reshape(S, D), A_wq, A_wk, A_wv, A_wo, A_beta.reshape(1, H), B_wqkv, B_wo)
        return out.reshape(A_x.shape)
    return fn


_fused = make()


@jax.jit
def pallas_interleave_layers__memory_aug_infini_attn__sliding_local_dilated__prompt_kernel(
    A_x: jax.Array,
    A_wq: jax.Array,
    A_wk: jax.Array,
    A_wv: jax.Array,
    A_wo: jax.Array,
    A_beta: jax.Array,
    B_x: jax.Array,
    B_wqkv: jax.Array,
    B_wo: jax.Array,
):
    return _fused(A_x, A_wq, A_wk, A_wv, A_wo, A_beta, B_x, B_wqkv, B_wo)
```

```python
import functools
import math

import jax
import jax.numpy as jnp
from jax import lax
from jax.experimental import pallas as pl
from jax.experimental.pallas import tpu as pltpu

BF = jnp.bfloat16
F32 = jnp.float32
U32 = jnp.uint32
I32 = jnp.int32

S = 2048
D = 1024
HD = D // 2
H = 32
DH = 32
SEG = 512
NSEG = S // SEG
NG = D // 128
NP = NG // 2
TB = 256
WIN = 8
DIL = 2
HALO = 16
NSLOT = 6
NSEM = 16
LOG2E = math.log2(math.e)
MASKED = -1e9 * LOG2E
QSCALE = DH ** -0.5 * LOG2E


def _dot(a, b):
    return jnp.dot(a, b, preferred_element_type=F32)


def _dot_nt(a, b):
    return lax.dot_general(a, b, (((1,), (1,)), ((), ())), preferred_element_type=F32)


def _phi(t):
    return jnp.where(t > 0, t + 1.0, jnp.exp(t))


def _recip(x):
    r = pltpu.reciprocal(x, approx=True)
    return r * (2.0 - x * r)


def _cat(xs, axis):
    return xs[0] if len(xs) == 1 else jnp.concatenate(xs, axis=axis)


def _tree(op, xs):
    while len(xs) > 1:
        xs = [op(xs[i], xs[i + 1]) for i in range(0, len(xs), 2)]
    return xs[0]


def _tile(j):
    return slice(128 * j, 128 * j + 128)


def _first(a, b):
    del b
    return a


LHS7 = ((0, 3, jnp.add), (2, 3, jnp.add), (0, 0, _first), (3, 3, _first),
        (0, 1, jnp.add), (2, 0, jnp.subtract), (1, 3, jnp.subtract))


def _lhs7(*a):
    return [op(a[x], a[y]).astype(BF) for x, y, op in LHS7]


def _rhs7(b11, b12, b21, b22):
    f11, f12, f21, f22 = [b.astype(F32) for b in (b11, b12, b21, b22)]
    return [b.astype(BF) for b in (f11 + f22, b11, f12 - f22, f21 - f11, b22, f11 + f12, f21 + f22)]


class _Pacer:
    def __init__(self, tmp, step):
        self.tmp = tmp
        self.z = [step >> (10 + i) for i in range(5)]
        self.plan, self.due = {}, {}
        self.pending, self.ready = [], []
        self.count = 0

    def spread(self, fn, n, first, last, slack):
        for i in range(n):
            t = first + i * (last - first) / (n - 1)
            self.plan.setdefault(int(t), []).append((fn, i, t - int(t), slack and t + slack))

    def product(self, thunk):
        for fn, i, go, when in self.pending:
            done = fn(i, go)
            if when and done is not None:
                self.due.setdefault(int(when), []).append((when - int(when), done))
        self.pending = []
        self.ready += self.due.pop(self.count, [])
        y = thunk()
        for fn, i, frac, when in self.plan.pop(self.count, []):
            r = 8 * int(frac * (y.shape[0] // 8))
            self.pending.append((fn, i, y[r:r + 8], when))
        self.count += 1
        return y

    def after(self, t, x):
        bits = pltpu.bitcast(x, U32) | (pltpu.bitcast(t, U32) & self.z[0].astype(U32))
        return pltpu.bitcast(bits, x.dtype)

    def lhs(self, words):
        if self.ready:
            n = words.shape[0] // 8
            heads = [words[8 * i:8 * i + 8, 0:128] for i in range(n)]
            for frac, t in self.ready:
                heads[int(frac * n)] = self.after(t, heads[int(frac * n)])
            words = _cat([_cat(heads, 0), words[:, 128:]], 1)
            self.ready = []
        return pltpu.bitcast(words, BF)

    def finish(self):
        assert not self.plan and not self.pending

    def strassen(self, prod, emit=None, between=None):
        def run(i):
            if between:
                between()
            return self.product(functools.partial(prod, i))
        m3 = run(2)
        rows = slice(0, m3.shape[0])

        def put(i, v):
            self.tmp[i][self.z[0], rows, :] = v

        def get(i, n):
            return self.tmp[i][self.z[n], rows, :]
        put(0, m3)
        put(1, run(0))
        put(2, run(6))
        put(3, run(1))
        m5 = run(4)
        c12 = get(0, 1) + m5
        emit(0, 1, c12) if emit else put(5, c12)
        put(4, (get(1, 1) + get(2, 1)) - m5)
        c22 = ((get(1, 2) - get(3, 2)) + get(0, 2)) + run(5)
        emit(1, 1, c22) if emit else put(6, c22)
        m4 = run(3)
        c21, c11 = get(3, 1) + m4, get(4, 1) + m4
        if emit:
            emit(1, 0, c21)
            emit(0, 0, c11)
            return None
        return c11, get(5, 1), c21, get(6, 1)


def _scratch():
    vm = pltpu.VMEM
    return dict(
        xio=vm((S, D), BF),
        xn_u=vm((7, SEG // 4, HD), U32),
        xc=vm((1, SEG, D), F32),
        mean=vm((1, SEG + 32, 128), F32),
        rstd=vm((1, SEG + 32, 128), F32),
        qvk_st=[vm((2, D, HD), BF)] * 3,
        wo_st=vm((D + 16, D), BF),
        wqkv_st=vm((4, D, D), BF),
        wob_st=vm((D + 16, D), BF),
        perm=[vm((NG, 264, 128), U32)] * 3,
        wqvt_u=vm((NP, 7, 128, HD), U32),
        wk_u=vm((2, 7, HD // 2, 256), U32),
        wqkv_u=vm((4, 7, HD // 2, HD), U32),
        wob_u=vm((7, HD // 2, HD), U32),
        wob_rows=vm((2, 34 * H, 128), F32),
        oa_u=vm((2, 7, SEG // 4, 256), U32),
        mem=vm((NG, 144, 128), F32),
        gate=vm((H, 8, 128), F32),
        bias=vm((3, 64, 128), F32),
        zsum=vm((2, 8, 256), F32),
        recall=vm((4, 144, SEG), F32),
        kqs=[vm((2 * NG, HALO + TB, 128), F32)] * 2,
        vbs=[vm((NG + 2, HALO + TB, 128), F32)] * 2,
        pbs=[vm((WIN, TB, 128), F32)] * 2,
        obs_u=[vm((7, TB // 4, HD), U32)] * 2,
        sems=pltpu.SemaphoreType.DMA((NSEM,)),
        sbufs=[vm((1, 4, SEG, 128), F32)] * NSLOT,
        tmp=[vm((1, 256, 128), F32)] * 7,
        tiles=[vm((1, 128, 128), F32)] * 4,
        qt=[vm((2, 128, SEG), BF)] * 2,
        pqt=[vm((2, 128, SEG), BF)] * 2,
        vt=[vm((2, 128, SEG), BF)] * 2,
        kk=[vm((1, SEG, 256), BF)] * 2,
        pk=[vm((1, SEG, 256), BF)] * 2,
        wo_u=[vm((7, HD // 4, 256), U32)] * NP,
        beta=vm((1, H), BF),
    )


def _kernel(x_hbm, wq_hbm, wk_hbm, wv_hbm, wo_hbm, beta_hbm, wqkv_hbm, wob_hbm, out_hbm,
            xio, xn_u, xc, mean, rstd, qvk_st, wo_st, wqkv_st, wob_st, perm,
            wqvt_u, wk_u, wqkv_u, wob_u, wob_rows, oa_u, mem, gate, bias, zsum, recall,
            kqs, vbs, pbs, obs_u, sems, sbufs, tmp, tiles, qt, pqt, vt, kk, pk, wo_u, beta):
    oa, xn, wqvt, wk, wqkv, wob = [r.bitcast(BF) for r in (oa_u, xn_u, wqvt_u, wk_u, wqkv_u, wob_u)]
    wo = [r.bitcast(BF) for r in wo_u]
    obs = [r.bitcast(BF) for r in obs_u]

    def segment(s):
        return xio.at[pl.ds(pl.multiple_of(s * SEG, SEG), SEG)]

    sem_ids = iter(range(NSEM))

    def fetch(src, dst):
        return pltpu.make_async_copy(src, dst, sems.at[next(sem_ids)])

    x_in = [fetch(x_hbm.at[pl.ds(r, n)], xio.at[pl.ds(r, n)]) for r, n in ((0, TB), (TB, TB), (SEG, S - SEG))]
    w_in = [[fetch(src.at[:, pl.ds(HD * i, HD)], dst.at[i]) for src, dst in zip((wq_hbm, wv_hbm, wk_hbm), qvk_st)]
            for i in range(2)]
    late_in = [x_in[2], fetch(wo_hbm, wo_st.at[pl.ds(0, D)]), fetch(wob_hbm, wob_st.at[pl.ds(0, D)])]
    late_in += [fetch(wqkv_hbm.at[:, pl.ds(D * i, D)], wqkv_st.at[i]) for i in range(3)]
    beta_in = fetch(beta_hbm, beta)
    out_sem = sems.at[next(sem_ids)]

    def out_copy(s, c):
        rows = pl.ds(pl.multiple_of(s * SEG, SEG) + TB * c, TB)
        return pltpu.make_async_copy(xio.at[rows], out_hbm.at[rows], out_sem)

    def norm_mean(z, s, i, go):
        if go is not None:
            mean[z[1], SEG:SEG + 8, :] = go
        rows = slice(8 * i, 8 * i + 8)
        m = jnp.mean(segment(s)[rows, :].astype(F32), axis=-1, keepdims=True)
        mean[z[0], rows, :] = jnp.broadcast_to(m, (8, 128))

    def norm_var(z, s, i, go):
        mean[z[0], SEG:SEG + 8, :] = go
        rows = slice(8 * i, 8 * i + 8)
        x = segment(s + z[0])[rows, :].astype(F32) - _cat([mean[z[1], rows, :]] * NG, 1)
        xc[z[0], rows, :] = x
        v = jnp.mean(x * x, axis=-1, keepdims=True)
        rstd[z[0], rows, :] = lax.rsqrt(jnp.broadcast_to(v, (8, 128)) + 1e-5)
        return rstd[z[2], rows, :]

    def norm_store(z, i, go):
        rstd[z[0], SEG:SEG + 8, :] = go
        i, e = divmod(i, 4)
        c, r = divmod(16 * i, 128)
        a = [xc[z[1], o:o + 16, _tile(j)] * rstd[z[1], o:o + 16, :]
             for o in (TB * c + r, TB * c + r + 128) for j in (e, 4 + e)]
        for n, v in enumerate(_lhs7(*a)):
            xn[n, 16 * i:16 * i + 16, _tile(e)] = v
        return xn_u[z[2], 8 * i:8 * i + 8, _tile(e)]

    for cp in (beta_in, x_in[0], x_in[1], w_in[0][0]):
        cp.start()

    key = lax.broadcasted_iota(I32, (64, 128), 0)
    col = lax.broadcasted_iota(I32, (64, 128), 1)
    for i, query in enumerate((col, col ^ 64, col & 63)):
        bias[i] = jnp.where(key <= query, 0.0, MASKED)
    beta_in.wait()
    diag = lax.broadcasted_iota(I32, (H, H), 0) == lax.broadcasted_iota(I32, (H, H), 1)
    b_row = jnp.broadcast_to(beta[...].astype(F32), (H, H))
    b_col = jnp.sum(jnp.where(diag, b_row, 0.0), axis=1, keepdims=True)
    g_all = jax.nn.sigmoid(jnp.broadcast_to(b_col, (H, 128)))
    for h in range(H):
        gate[h] = jnp.broadcast_to(g_all[h:h + 1], (8, 128))

    def clear(i, c):
        wqkv_st[3, pl.ds(pl.multiple_of(i * 128, 128), 128), :] = jnp.zeros((128, D), BF)
        return c
    lax.fori_loop(0, D // 128, clear, 0)

    def first_norm(i, c):
        r = (i >> 1) * TB + (i & 1) * 64
        a = []
        for o in (0, 128):
            x = xio[pl.ds(pl.multiple_of(r + o, 64), 64), :].astype(F32)
            x = x - jnp.mean(x, axis=-1, keepdims=True)
            x = x * lax.rsqrt(jnp.mean(x * x, axis=-1, keepdims=True) + 1e-5)
            a += [x[:, :HD], x[:, HD:]]
        for n, v in enumerate(_lhs7(*a)):
            xn[n, pl.ds(pl.multiple_of(i * 64, 64), 64), :] = v
        return c
    for i in range(2):
        x_in[i].wait()
        w_in[0][1 + i].start()
        lax.fori_loop(2 * i, 2 * i + 2, first_norm, 0)

    def head_setup(it):
        for m in range(2):
            for i in range(2):
                pl.when(it == i)(w_in[i][m].wait)
            if m == 1:
                @pl.when(it == 0)
                def _():
                    for cp in w_in[1]:
                        cp.start()
            for e in range(2):
                t = qvk_st[m][it, :, 256 * e:256 * e + 256].T
                for i, b in enumerate(_rhs7(t[:128, :HD], t[128:, :HD], t[:128, HD:], t[128:, HD:])):
                    wqvt[2 * it + e, i, _tile(m), :] = b
        for i in range(2):
            pl.when(it == i)(w_in[i][2].wait)

        @pl.when(it == 0)
        def _():
            for cp in late_in:
                cp.start()

        def wk_body(i, c):
            for o in range(0, 128, 16):
                r = pl.multiple_of(i * 128, 128) + o
                halves = [qvk_st[2][it, pl.ds(r + k, 16), :] for k in (0, HD)]
                blocks = [_cat([w[:, _tile(e)], w[:, _tile(2 + e)]], 1) for w in halves for e in range(2)]
                for n, b in enumerate(_rhs7(*blocks)):
                    wk[it, n, pl.ds(r, 16), :] = b
            return c
        lax.fori_loop(0, HD // 128, wk_body, 0)

    def prep_out(z, n, r, go):
        src = 256 * (r // 8) + 16 * (r % 8)
        if go is not None:
            wo_st[D:D + 8, 0:128] = go.astype(BF)
            src = pl.multiple_of(z[1], 16) + src
        blocks = [wo_st[pl.ds(src + o, 16), _tile(2 * n + e)] for o in (0, 128) for e in range(2)]
        for m, b in enumerate(_rhs7(*blocks)):
            wo[n][m, 16 * (r % 16):16 * (r % 16) + 16, _tile(r // 16)] = b
        return None if go is None else wo_u[n][z[2], 0:8, 0:128]

    def late_setup():
        for cp in late_in:
            cp.wait()
        for n in range(2):
            for r in range(32):
                prep_out(None, n, r, None)

    lane = lax.broadcasted_iota(I32, (8, 128), 1)

    def prep_spread(z, s, it, i, go):
        perm[0][z[1], 256:264, :] = pltpu.bitcast(go, U32)
        g, k = divmod(i, 4)
        rows = pl.ds(pl.multiple_of(256 * it, 256) + (k >> 1) * HD + (k & 1) * 128, 128)
        w = pltpu.bitcast(wqkv_st[(s - 1) & 3, rows, _tile(g)], U32)
        src = 32 * (lane & 3) + 4 * (((lane >> 4) - g) & 7) + ((lane & 15) >> 2)
        perm[0][z[0] + g, 64 * k:64 * k + 64, :] = jnp.take_along_axis(w, _cat([src] * 8, 0), axis=1)
        return perm[0][z[2] + g, 64 * k:64 * k + 8, :]

    def prep_exchange(z, i, go):
        perm[0][z[0], 256:264, :] = pltpu.bitcast(go, U32)
        u = [perm[0][z[1] + (-j) % NG, 8 * i:8 * i + 8, :] for j in range(NG)]
        for bit in (1, 2, 4):
            m = (lane & (16 * bit)) != 0
            u = [jnp.where(m, u[(j - bit) % NG], u[j]) for j in range(NG)]
        for j in range(NG):
            perm[1][z[0] + j, 8 * i:8 * i + 8, :] = u[j]
        return perm[1][z[2], 8 * i:8 * i + 8, :]

    def prep_collect(z, i, go):
        perm[1][z[0], 256:264, :] = pltpu.bitcast(go, U32)
        j, k = divmod(i, 4)
        src = 16 * (((lane >> 2) + j) & 7) + 4 * (lane >> 5) + (lane & 3)
        w = perm[1][z[1] + j, 64 * k:64 * k + 64, :]
        perm[2][z[0] + j, 64 * k:64 * k + 64, :] = jnp.take_along_axis(w, _cat([src] * 8, 0), axis=1)
        return perm[2][z[2] + j, 64 * k:64 * k + 8, :]

    def prep_combine(z, s, it, i, go):
        perm[2][z[0], 256:264, :] = pltpu.bitcast(go, U32)
        r, p = divmod(i, NP)
        w = [pltpu.bitcast(perm[2][z[1] + 2 * p + e, o + 8 * r:o + 8 * r + 8, :], BF)
             for o in (0, 128) for e in range(2)]
        rows = pl.ds(pl.multiple_of(256 * it, 256) + 16 * r, 16)
        for n, b in enumerate(_rhs7(*w)):
            wqkv[s, n, rows, _tile(p)] = b
        return pltpu.bitcast(wqkv[z[2] + s, 0, rows, _tile(p)], U32)

    def prep_wob_rows(z, s, h, go):
        wob_st[D:D + 8, 0:128] = go.astype(BF)
        w = wob_st[32 * h:32 * h + 32, pl.ds(pl.multiple_of(s * 256, 256), 256)].astype(F32)
        for e in range(2):
            wob_rows[z[0] + e, 33 * h:33 * h + 32, :] = w[:, _tile(e)]
        return wob_rows[z[2], 0:8, :]

    def prep_wob(z, s, i, go):
        wob_rows[z[0], 33 * H:33 * H + 8, :] = go
        d, e = divmod(i, 2)
        blocks = [wob_rows[z[1] + c, pl.ds(33 * 16 * e + dd, 16, stride=33), :]
                  for dd in (d, d + DH // 2) for c in range(2)]
        cols = pl.ds(pl.multiple_of(s * 128, 128), 128)
        for n, b in enumerate(_rhs7(*blocks)):
            wob[n, 16 * i:16 * i + 16, cols] = b
        return wob_u[z[2], 0:8, cols]

    def add_residual(s, r0, n, blocks):
        seg = segment(s)
        for y, o in ((_cat(blocks[:2], 1), 0), (_cat(blocks[2:], 1), 128)):
            for i in range(y.shape[0] // 128):
                view = (slice(r0 + TB * i + o, r0 + TB * i + o + 128), slice(256 * n, 256 * n + 256))
                seg[view] = (seg[view].astype(F32) + y[_tile(i)]).astype(BF)

    upper = lane >= 64

    def project(pc, it, e, between=None):
        z = pc.z
        c11, c12, c21, c22 = pc.strassen(
            lambda i: _dot(pc.lhs(xn_u[i]), wk[it, i, :, _tile(e)]), between=between)
        total = []
        for k, r0 in ((_cat([c11, c12], 1), 0), (_cat([c21, c22], 1), 128)):
            part = None
            for i in range(2):
                rows = slice(TB * i + r0, TB * i + r0 + 128)
                kk[e][z[0], rows, :] = k[_tile(i)].astype(BF)
                f = _phi(k[_tile(i)])
                pieces = []
                for r in range(0, 128, 8):
                    part = f[r:r + 8] if part is None else part + f[r:r + 8]
                    pieces.append(pc.after(part, f[r:r + 8]) if r % 32 == 24 else f[r:r + 8])
                pk[e][z[0], rows, :] = _cat(pieces, 0).astype(BF)
            total.append(part)
        zsum[z[0] + e] = jnp.broadcast_to(jnp.sum(total[0] + total[1], axis=0, keepdims=True), (8, 256))
        for c in range(2):
            c11, c12, c21, c22 = pc.strassen(
                lambda i: _dot_nt(pc.lhs(wqvt_u[z[c] + 2 * it + e, i]), xn[i, _tile(c), :]), between=between)
            for o, y in enumerate((_cat([c11, c21], 1), _cat([c12, c22], 1))):
                q, lanes, g = y[:128], slice(TB * c, TB * c + TB), z[0] + o
                for h in range(4):
                    qh = q[32 * h:32 * h + 32] * QSCALE
                    if h % 2:
                        qh = _cat([pltpu.roll(qh[:, _tile(i)], 64, 1) for i in range(2)], 1)
                    qt[e][g, 32 * h:32 * h + 32, lanes] = qh.astype(BF)
                pqt[e][g, :, lanes] = _phi(q).astype(BF)
                vt[e][g, :, lanes] = y[128:].astype(BF)

    def scores(z, g, j, t, sbuf, mx):
        zero = jnp.zeros((32, 128), BF)
        q = [qt[g // 2][z[1 + t] + g % 2, 32 * h:32 * h + 32, _tile(j)] for h in range(4)]
        n = 64 if t == j else 128
        rows = slice(128 * t, 128 * t + n)
        s = _dot(kk[g // 2][z[1], rows, _tile(g % 2)],
                 _cat([_cat([q[h] if i == h else zero for i in range(4)], 0) for h in range(4)], 1))
        for h in range(4):
            sh = s[:, _tile(h)]
            if t == j:
                sh = sh + bias[h & 1]
            sbuf[z[0], h, rows, :] = sh
            for i in range(0, n, 8):
                mx[h] = sh[i:i + 8] if mx[h] is None else jnp.maximum(mx[h], sh[i:i + 8])
        if t < j:
            return
        q = [pltpu.bitcast(jnp.where(_cat([upper == (h % 2 == 0)] * 2, 0), pltpu.bitcast(q[h], U32),
                                     jnp.zeros((16, 128), U32)), BF) for h in range(4)]
        rows = slice(128 * t + 64, 128 * t + 128)
        s = _dot(kk[g // 2][z[1], rows, _tile(g % 2)],
                 _cat([_cat([q[0], q[1], zero, zero], 0), _cat([zero, zero, q[2], q[3]], 0)], 1))
        for h in (0, 2):
            sh = s[:, _tile(h // 2)] + bias[2]
            sbuf[z[0], h, rows, :] = sh
            m = functools.reduce(jnp.maximum, [sh[i:i + 8] for i in range(0, 64, 8)])
            mx[h] = jnp.where(upper, jnp.maximum(mx[h], m), mx[h])
            mx[h + 1] = jnp.where(upper, mx[h + 1], jnp.maximum(mx[h + 1], m))
        for h in range(4):
            mx[h] = jnp.broadcast_to(jnp.max(mx[h], axis=0, keepdims=True), (8, 128))

    def attend(pc, g, j, t, sbuf, mx, acc, tot):
        z = pc.z

        def probs(h, r, m):
            p = jnp.exp2(sbuf[z[1], h, r:r + 64, :] - _cat([m] * 8, 0))
            return p, _tree(jnp.add, [p[i:i + 8] for i in range(0, 64, 8)])
        for h in range(4):
            if t < j:
                hi, part = probs(h, 128 * t + 64, mx[h])
            else:
                if h % 2 == 0:
                    shared = probs(h, 128 * t + 64, jnp.where(upper, mx[h], mx[h + 1]))
                mine = upper == (h % 2 == 0)
                hi, part = jnp.where(_cat([mine] * 8, 0), shared[0], 0.0), jnp.where(mine, shared[1], 0.0)
            tot[h] = part if tot[h] is None else tot[h] + part
            hi = [pc.after(tot[h], hi[0:8]), hi[8:]]
            lo, part = probs(h, 128 * t, mx[h])
            tot[h] = tot[h] + part
            p = _cat([pc.after(tot[h], lo[0:8]), lo[8:]] + hi, 0)
            r = _dot(vt[g // 2][z[1] + g % 2, 32 * h:32 * h + 32, _tile(t)], p.astype(BF))
            acc[h] = r if acc[h] is None else acc[h] + r

    def memory_read(z, it, g):
        recall[z[0] + g] = _dot(mem[4 * it + g].astype(BF), pqt[g // 2][z[1] + g % 2])

    def memory_update(z, it, g):
        upd = _dot(vt[g // 2][z[1] + g % 2], pk[g // 2][z[1], :, _tile(g % 2)])
        upd = _cat([upd, zsum[z[1] + g // 2, :, _tile(g % 2)]], 0)
        head = lane >> 5
        keep = _cat([head == r // 4 for r in range(16)] + [head == lax.broadcasted_iota(I32, (8, 128), 0)], 0)
        mem[4 * it + g, 0:136, :] = mem[z[1] + 4 * it + g, 0:136, :] + jnp.where(keep, upd, 0.0)

    def gated(z, it, g, j, acc, tot):
        inv_den = _recip(recall[z[1] + g, 128:136, _tile(j)] + 1e-6)
        outs = []
        for h in range(4):
            gt = gate[16 * it + 4 * g + h]
            c_dot = (1.0 - gt) * _recip(jnp.broadcast_to(jnp.sum(tot[h], axis=0, keepdims=True), (8, 128)))
            c_mem = gt * jnp.broadcast_to(inv_den[h:h + 1], (8, 128))
            local = acc[h] * _cat([c_dot] * 4, 0)
            if h % 2:
                local = pltpu.roll(local, 64, 1)
            outs.append(local + recall[z[1] + g, 32 * h:32 * h + 32, _tile(j)] * _cat([c_mem] * 4, 0))
        return _cat(outs, 0)

    def heads_step(l, s, it, carry):
        pl.when((l == 0) & (s == 0))(functools.partial(head_setup, it))
        pc = _Pacer(tmp, it)
        z = pc.z
        pc.spread(functools.partial(prep_spread, z, s, it), 32, 0.86, 4.5, 1.84)
        pc.spread(functools.partial(prep_exchange, z), 32, 5.04, 8.5, 1.2)
        pc.spread(functools.partial(prep_collect, z), 32, 9.54, 12.2, 1.5)
        pc.spread(functools.partial(prep_combine, z, s, it), 64, 14, 22, 1.2)
        order = ((0, 3), (0, 2), (1, 3), (1, 2), (0, 1), (1, 1), (0, 0), (1, 0))
        items = [(2 * p + e, j) for p in range(2) for e, j in order]
        units = [(n, g, j, t) for n, (g, j) in enumerate(items) for t in range(j + 1)]
        state = [([None] * 4, [None] * 4, [None] * 4) for _ in items]
        last = {n: k for k, (n, *_) in enumerate(units)}
        seen = []

        def consume(n, g, j, t):
            attend(pc, g, j, t, sbufs[n % NSLOT], *state[n])
            if t < j:
                return
            o = gated(z, it, g, j, *state[n][1:])
            me = 2 * (j & 1) + (g & 1)
            seen.append(me)
            if len(seen) < 4:
                tiles[me][z[0]] = o
            for i, (x, y, op) in enumerate(LHS7):
                if me in (x, y) and x in seen and y in seen:
                    a, b = [o if q == me else tiles[q][z[1 + me]] for q in (x, y)]
                    oa[it, i, _tile(j // 2), _tile(g // 2)] = op(a, b).astype(BF).T
            if len(seen) == 4:
                seen.clear()

        def rounds():
            reads = (0, 1, 24, 30)
            done, k, updated = 0, 0, 0
            while done < len(units):
                if k in reads:
                    memory_read(z, it, reads.index(k))
                if k < len(units):
                    n, g, j, t = units[k]
                    scores(z, g, j, t, sbufs[n % NSLOT], state[n][0])
                else:
                    memory_update(z, it, updated)
                    updated += 1
                for _ in range(2 if k >= len(units) - 4 else 1):
                    if done < len(units) and last[units[done][0]] + 2 <= k:
                        consume(*units[done])
                        done += 1
                k += 1
                yield
            for g in range(updated, 4):
                memory_update(z, it, g)

        project(pc, it, 0)
        attention = rounds()
        slots = iter(range(21))

        def between():
            if next(slots) >= 5:
                next(attention)
        project(pc, it, 1, between)
        pc.finish()
        for _ in attention:
            pass
        return carry

    def infini_step(l, s, carry):
        lax.fori_loop(0, 2, functools.partial(heads_step, l, s), 0)
        pl.when((l == 0) & (s == 0))(late_setup)
        pc = _Pacer(tmp, s)
        z = pc.z
        nxt = (s + 1) & (NSEG - 1)
        for i in range(SEG // 8):
            norm_mean(z, nxt, i, None)
        pc.spread(functools.partial(norm_var, z, nxt), SEG // 8, 0, 5.9, 0)
        pc.spread(functools.partial(norm_store, z), SEG // 8, 7, 24.62, 1.3)
        for n in range(2, NP):
            pc.spread(functools.partial(prep_out, z, n), 32, 7 * n - 8, 7 * n - 2.3, 1.2)
        pc.spread(functools.partial(prep_wob_rows, z, s), H, 6, 11.44, 1.5)
        pc.spread(functools.partial(prep_wob, z, s), DH, 14, 24.34, 1.2)
        for n in range(NP):
            add_residual(s, 0, n, pc.strassen(lambda i: _dot(
                pc.lhs(_cat([oa_u[0, i], oa_u[1, i]], 1)),
                _cat([wo[n][z[1] + i, :, _tile(e)] for e in range(2)], 0))))
        pc.finish()
        return carry

    def window_step(l, s, carry):
        pc = _Pacer(tmp, s)
        z = pc.z
        held = {}

        def taps(ref, j, r, n):
            out = [None] * WIN
            for a in range(WIN // 2):
                slab = ref[z[1] + j, pl.ds(HALO + r - 8 - DIL * a, n + 8), :]
                out[a] = slab[8:]
                out[a + 4] = slab[:n]
            return out

        def probs(c, i, go):
            kqs[c][z[0] + NG, 0:8, :] = go
            i, step = divmod(i, 4)
            r = (i >> 1) * 8 + (i & 1) * 128
            acc = held.pop(("k", c), [None] * WIN)
            for j in (2 * step, 2 * step + 1):
                q = kqs[c][z[1] + NG + j, HALO + r:HALO + r + 8, :]
                for w, k in enumerate(taps(kqs[c], j, r, 8)):
                    acc[w] = q * k if j == 0 else acc[w] + q * k
            if step < 3:
                held["k", c] = acc
                return None
            acc = [a + pltpu.roll(a, 64, 1) for a in acc]
            acc = [a + pltpu.roll(a, 32, 1) for a in acc]
            for w in range(WIN):
                if c == 0 and r < DIL * w:
                    pos = s * SEG + r + lax.broadcasted_iota(I32, (8, 128), 0)
                    acc[w] = jnp.where(pos >= DIL * w, acc[w], MASKED)
            m = _tree(jnp.maximum, acc)
            p = [jnp.exp2(a - m) for a in acc]
            inv = _recip(_tree(jnp.add, p))
            for w in range(WIN):
                pbs[c][z[0] + w, r:r + 8, :] = p[w] * inv
            return pbs[c][z[2], r:r + 8, :]

        def values(c, i, go):
            i, step = divmod(i, 5)
            r, e = 16 * (i // 4), i % 4
            if step == 4:
                for n, v in enumerate(_lhs7(*held.pop(("v", c)))):
                    obs[c][z[0] + n, r:r + 16, _tile(e)] = v
                return pltpu.bitcast(obs[c][z[2], r:r + 16, _tile(e)], U32)
            vbs[c][z[0] + NG, 0:8, :] = go
            o, j = r + 128 * (step >> 1), e + 4 * (step & 1)
            y = None
            for w, v in enumerate(taps(vbs[c], j, o, 16)):
                t = pbs[c][z[1 + e] + w, o:o + 16, :] * v
                y = t if y is None else y + t
            held.setdefault(("v", c), []).append(y)
            return pltpu.bitcast(y[0:8], U32) | pltpu.bitcast(y[8:16], U32)

        nxt = (s + 1) & (NSEG - 1)
        pc.spread(functools.partial(norm_mean, z, nxt), SEG // 8, 1, 20, 0)
        pc.spread(functools.partial(norm_var, z, nxt), SEG // 8, 21, 53, 4)
        pc.spread(functools.partial(probs, 0), 4 * TB // 8, 58.36, 106, 6.45)
        pc.spread(functools.partial(values, 0), 5 * TB // 8, 147.21, 165.5, 2.28)
        pc.spread(functools.partial(probs, 1), 4 * TB // 8, 112, 146, 5.5)
        pc.spread(functools.partial(values, 1), 5 * TB // 8, 168, 194.33, 2)
        pc.spread(functools.partial(norm_store, z), SEG // 8, 195.9, 214.54, 1.52)

        def project_window(c, part, p):
            refs = vbs if part == 2 else kqs

            def emit(half, e, y):
                if part == 0:
                    y = y * QSCALE
                j = z[0] + 2 * p + e
                refs[c][j + (NG if part == 0 else 0), HALO + 128 * half:HALO + 128 * half + 128, :] = y
                if part > 0 and c == 0 and half == 1:
                    refs[1][j, 0:HALO, :] = y[128 - HALO:]
            pc.strassen(lambda i: _dot(pc.lhs(xn_u[i, 64 * c:64 * c + 64, :]), wqkv[part + 1, i, :, _tile(p)]), emit)

        for c, part in ((0, 0), (0, 1), (1, 0), (1, 1), (0, 2), (1, 2)):
            for p in range(NP):
                project_window(c, part, p)
        for c in range(2):
            for n in range(NP):
                add_residual(s, TB * c, n, pc.strassen(
                    lambda i: _dot(pc.lhs(obs_u[c][z[1 + n] + i]), wob[i, :, _tile(n)])))
            pl.when(l == 1)(out_copy(s, c).start)
        pc.finish()
        for refs in (kqs, vbs):
            for j in range(NG):
                refs[0][z[0] + j, 0:HALO, :] = refs[1][z[2] + j, TB:TB + HALO, :]
        return carry

    def layer_pair(l, carry):
        mem[...] = jnp.zeros(mem.shape, F32)
        lax.fori_loop(0, NSEG, functools.partial(infini_step, l), 0)
        for refs in (kqs, vbs):
            refs[0][0:NG, 0:HALO, :] = jnp.zeros((NG, HALO, 128), F32)
        lax.fori_loop(0, NSEG, functools.partial(window_step, l), 0)
        return carry
    lax.fori_loop(0, 2, layer_pair, 0)
    pltpu.make_async_copy(xio, out_hbm, out_sem).wait()


@jax.jit
def pallas_interleave_layers__memory_aug_infini_attn__sliding_local_dilated__prompt_kernel(
    A_x: jax.Array,
    A_wq: jax.Array,
    A_wk: jax.Array,
    A_wv: jax.Array,
    A_wo: jax.Array,
    A_beta: jax.Array,
    B_x: jax.Array,
    B_wqkv: jax.Array,
    B_wo: jax.Array,
):
    del B_x
    hbm = pl.BlockSpec(memory_space=pl.ANY)
    out = pl.pallas_call(
        _kernel,
        out_shape=jax.ShapeDtypeStruct((S, D), BF),
        in_specs=[hbm] * 8,
        out_specs=hbm,
        scratch_shapes=list(_scratch().values()),
        compiler_params=pltpu.CompilerParams(vmem_limit_bytes=110 * 2 ** 20),
        name="fused_layers",
    )(A_x.reshape(S, D), A_wq, A_wk, A_wv, A_wo, A_beta.reshape(1, H), B_wqkv, B_wo)
    return out.reshape(A_x.shape)
```

```python
import functools
import math

import jax
import jax.numpy as jnp
from jax import lax
from jax.experimental import pallas as pl
from jax.experimental.pallas import tpu as pltpu

BF = jnp.bfloat16
F32 = jnp.float32
U32 = jnp.uint32
I32 = jnp.int32

S = 2048
D = 1024
HD = D // 2
H = 32
DH = 32
SEG = 512
NSEG = S // SEG
NG = D // 128
NP = NG // 2
TB = 256
WIN = 8
DIL = 2
HALO = 16
NSLOT = 6
NSEM = 16
LOG2E = math.log2(math.e)
MASKED = -1e9 * LOG2E
QSCALE = DH ** -0.5 * LOG2E


def _dot(a, b):
    return jnp.dot(a, b, preferred_element_type=F32)


def _dot_nt(a, b):
    return lax.dot_general(a, b, (((1,), (1,)), ((), ())), preferred_element_type=F32)


def _phi(t):
    return jnp.where(t > 0, t + 1.0, jnp.exp(t))


def _recip(x):
    r = pltpu.reciprocal(x, approx=True)
    return r * (2.0 - x * r)


def _cat(xs, axis):
    return xs[0] if len(xs) == 1 else jnp.concatenate(xs, axis=axis)


def _tree(op, xs):
    while len(xs) > 1:
        xs = [op(xs[i], xs[i + 1]) for i in range(0, len(xs), 2)]
    return xs[0]


def _tile(j):
    return slice(128 * j, 128 * j + 128)


def _first(a, b):
    del b
    return a


LHS7 = ((0, 3, jnp.add), (2, 3, jnp.add), (0, 0, _first), (3, 3, _first),
        (0, 1, jnp.add), (2, 0, jnp.subtract), (1, 3, jnp.subtract))


def _lhs7(*a):
    return [op(a[x], a[y]).astype(BF) for x, y, op in LHS7]


def _rhs7(b11, b12, b21, b22):
    f11, f12, f21, f22 = [b.astype(F32) for b in (b11, b12, b21, b22)]
    return [b.astype(BF) for b in (f11 + f22, b11, f12 - f22, f21 - f11, b22, f11 + f12, f21 + f22)]


class _Zeros:
    def __init__(self, step):
        self.cache = {(i, 0): step >> (10 + i) for i in range(6)}

    def __getitem__(self, key):
        key = key if isinstance(key, tuple) else (key, 0)
        if key not in self.cache:
            self.cache[key] = self.cache[key[0], 0] + key[1]
        return self.cache[key]


def _bits(x):
    return x if x.dtype == U32 else pltpu.bitcast(x, U32)


class _Pacer:
    def __init__(self, tmp, step):
        self.tmp = tmp
        self.z = _Zeros(step)
        self.no_bits = jnp.full((8, 128), self.z[0].astype(U32))
        self.plan, self.due = {}, {}
        self.pending, self.ready = [], []
        self.count = 0

    def spread(self, fn, n, first, last, slack):
        for i in range(n):
            t = first + i * (last - first) / (n - 1)
            self.plan.setdefault(int(t), []).append((fn, i, t - int(t), slack and t + slack))

    def product(self, thunk):
        for fn, i, go, when in self.pending:
            done = fn(i, go)
            if when and done is not None:
                self.due.setdefault(int(when), []).append((when - int(when), done))
        self.pending = []
        self.ready += self.due.pop(self.count, [])
        y = thunk()
        for fn, i, frac, when in self.plan.pop(self.count, []):
            r = 8 * int(frac * (y.shape[0] // 8))
            self.pending.append((fn, i, y[r:r + 8], when))
        self.count += 1
        return y

    def after(self, t, x):
        bits = _bits(x) | (_bits(t) & _cat([self.no_bits] * (x.shape[1] // 128), 1))
        return bits if x.dtype == U32 else pltpu.bitcast(bits, x.dtype)

    def lhs(self, words):
        if self.ready:
            n = words.shape[0] // 8
            heads = [words[8 * i:8 * i + 8, 0:128] for i in range(n)]
            for frac, t in self.ready:
                heads[int(frac * n)] = self.after(t, heads[int(frac * n)])
            words = _cat([_cat(heads, 0), words[:, 128:]], 1)
            self.ready = []
        return pltpu.bitcast(words, BF)

    def finish(self):
        assert not self.plan and not self.pending

    def strassen(self, prod, emit=None, emit_col=None, between=None):
        def run(i):
            if between:
                between()
            return self.product(functools.partial(prod, i))
        m3 = run(2)
        rows = slice(0, m3.shape[0])

        def put(i, v):
            self.tmp[i][self.z[0], rows, :] = v

        def get(i, n):
            return self.tmp[i][self.z[n], rows, :]
        put(0, m3)
        put(1, run(0))
        put(2, run(6))
        put(3, run(1))
        m5 = run(4)
        c12 = get(0, 1) + m5
        emit(0, 1, c12) if emit else put(5, c12)
        put(4, (get(1, 1) + get(2, 1)) - m5)
        c22 = ((get(1, 2) - get(3, 2)) + get(0, 2)) + run(5)
        if emit_col:
            emit_col(1, _cat([get(5, 1), c22], 1))
        else:
            emit(1, 1, c22) if emit else put(6, c22)
        m4 = run(3)
        c21, c11 = get(3, 1) + m4, get(4, 1) + m4
        if emit_col:
            return emit_col(0, _cat([c11, c21], 1))
        if emit:
            emit(1, 0, c21)
            emit(0, 0, c11)
            return None
        return c11, get(5, 1), c21, get(6, 1)


def _scratch():
    vm = pltpu.VMEM
    return dict(
        xio=vm((S, D), BF),
        xn_u=vm((7, SEG // 4, HD), U32),
        xc=vm((1, SEG, D), F32),
        mean=vm((1, SEG + 32, 128), F32),
        rstd=vm((1, SEG + 32, 128), F32),
        qvk_st=[vm((2, D + 16, HD), BF)] * 3,
        wo_st=vm((D + 16, D), BF),
        wqkv_st=vm((4, D, D), BF),
        wob_st=vm((D + 16, D), BF),
        perm=[vm((NG, 264, 128), U32)] * 3,
        flip_u=vm((2, 136, D), U32),
        wqvt_u=[vm((2, 7, 128, HD), U32)] * 2,
        wk_u=[vm((2, 7, HD // 4, 256), U32)] * 2,
        wqkv_u=vm((4, 7, HD // 2, HD), U32),
        wob_u=vm((7, HD // 2, HD), U32),
        wob_rows=vm((2, 34 * H, 128), F32),
        oa_u=vm((2, 7, SEG // 4, 256), U32),
        mem=vm((NG, 144, 128), F32),
        gate=vm((H, 8, 128), F32),
        bias=vm((3, 64, 128), F32),
        zsum=vm((4, 8, 128), F32),
        recall=vm((4, 144, SEG), F32),
        kqs=[vm((2 * NG, HALO + TB, 128), F32)] * 2,
        vbs=[vm((NG + 2, HALO + TB, 128), F32)] * 2,
        pbs=[vm((WIN, TB, 128), F32)] * 2,
        obs_u=[vm((7, TB // 4, HD), U32)] * 2,
        sems=pltpu.SemaphoreType.DMA((NSEM,)),
        sbufs=[vm((1, 4, SEG, 128), F32)] * NSLOT,
        tmp=[vm((1, 256, 128), F32)] * 7,
        tiles=[vm((1, 128, 128), F32)] * 4,
        qt_u=[vm((2, 64, SEG), U32)] * 2,
        pqt=[vm((2, 128, SEG), BF)] * 2,
        vt_u=[vm((2, 64, SEG), U32)] * 2,
        kk_u=[vm((2, TB // 2, 256), U32)] * 2,
        pk_u=[vm((2, TB // 2, 256), U32)] * 2,
        wo_u=[vm((7, HD // 4, 256), U32)] * NP,
        beta=vm((1, H), BF),
    )


def _kernel(x_hbm, wq_hbm, wk_hbm, wv_hbm, wo_hbm, beta_hbm, wqkv_hbm, wob_hbm, out_hbm,
            xio, xn_u, xc, mean, rstd, qvk_st, wo_st, wqkv_st, wob_st, perm, flip_u,
            wqvt_u, wk_u, wqkv_u, wob_u, wob_rows, oa_u, mem, gate, bias, zsum, recall,
            kqs, vbs, pbs, obs_u, sems, sbufs, tmp, tiles, qt_u, pqt, vt_u, kk_u, pk_u, wo_u, beta):
    oa, xn, flip, wqkv, wob = [r.bitcast(BF) for r in (oa_u, xn_u, flip_u, wqkv_u, wob_u)]
    wqvt, wk, wo, qt, vt, kk, pk, obs = [
        [r.bitcast(BF) for r in refs] for refs in (wqvt_u, wk_u, wo_u, qt_u, vt_u, kk_u, pk_u, obs_u)]

    def segment(s):
        return xio.at[pl.ds(pl.multiple_of(s * SEG, SEG), SEG)]

    sem_ids = iter(range(NSEM))

    def fetch(src, dst):
        return pltpu.make_async_copy(src, dst, sems.at[next(sem_ids)])

    x_in = [fetch(x_hbm.at[pl.ds(r, n)], xio.at[pl.ds(r, n)]) for r, n in ((0, TB), (TB, TB), (SEG, S - SEG))]
    w_in = [[fetch(src.at[:, pl.ds(HD * i, HD)], dst.at[i, pl.ds(0, D)]) for src, dst in zip((wq_hbm, wv_hbm, wk_hbm), qvk_st)]
            for i in range(2)]
    late_in = [x_in[2], fetch(wo_hbm, wo_st.at[pl.ds(0, D)]), fetch(wob_hbm, wob_st.at[pl.ds(0, D)])]
    late_in += [fetch(wqkv_hbm.at[:, pl.ds(D * i, D)], wqkv_st.at[i]) for i in range(3)]
    beta_in = fetch(beta_hbm, beta)
    out_sem = sems.at[next(sem_ids)]

    def out_copy(s, c):
        rows = pl.ds(pl.multiple_of(s * SEG, SEG) + TB * c, TB)
        return pltpu.make_async_copy(xio.at[rows], out_hbm.at[rows], out_sem)

    def norm_mean(z, s, i, go):
        if go is not None:
            mean[z[1], SEG:SEG + 8, :] = go
        rows = slice(8 * i, 8 * i + 8)
        m = jnp.mean(segment(s)[rows, :].astype(F32), axis=-1, keepdims=True)
        mean[z[0], rows, :] = jnp.broadcast_to(m, (8, 128))

    def norm_var(z, s, i, go):
        mean[z[0], SEG:SEG + 8, :] = go
        rows = slice(8 * i, 8 * i + 8)
        x = segment(s + z[0])[rows, :].astype(F32) - _cat([mean[z[1], rows, :]] * NG, 1)
        xc[z[0], rows, :] = x
        v = jnp.mean(x * x, axis=-1, keepdims=True)
        rstd[z[0], rows, :] = lax.rsqrt(jnp.broadcast_to(v, (8, 128)) + 1e-5)
        return rstd[z[2], rows, :]

    def norm_store(z, i, go):
        rstd[z[0], SEG:SEG + 8, :] = go
        i, e = divmod(i, 4)
        c, r = divmod(16 * i, 128)
        a = [xc[z[1], o:o + 16, _tile(j)] * rstd[z[1], o:o + 16, :]
             for o in (TB * c + r, TB * c + r + 128) for j in (e, 4 + e)]
        for n, v in enumerate(_lhs7(*a)):
            xn[n, 16 * i:16 * i + 16, _tile(e)] = v
        return xn_u[z[2], 8 * i:8 * i + 8, _tile(e)]

    for cp in (beta_in, x_in[0], x_in[1], w_in[0][0]):
        cp.start()

    key = lax.broadcasted_iota(I32, (64, 128), 0)
    col = lax.broadcasted_iota(I32, (64, 128), 1)
    for i, query in enumerate((col, col ^ 64, col & 63)):
        bias[i] = jnp.where(key <= query, 0.0, MASKED)
    beta_in.wait()
    diag = lax.broadcasted_iota(I32, (H, H), 0) == lax.broadcasted_iota(I32, (H, H), 1)
    b_row = jnp.broadcast_to(beta[...].astype(F32), (H, H))
    b_col = jnp.sum(jnp.where(diag, b_row, 0.0), axis=1, keepdims=True)
    g_all = jax.nn.sigmoid(jnp.broadcast_to(b_col, (H, 128)))
    for h in range(H):
        gate[h] = jnp.broadcast_to(g_all[h:h + 1], (8, 128))

    def clear(i, c):
        wqkv_st[3, pl.ds(pl.multiple_of(i * 128, 128), 128), :] = jnp.zeros((128, D), BF)
        return c
    lax.fori_loop(0, D // 128, clear, 0)

    def first_norm(i, c):
        r = (i >> 1) * TB + (i & 1) * 64
        a = []
        for o in (0, 128):
            x = xio[pl.ds(pl.multiple_of(r + o, 64), 64), :].astype(F32)
            x = x - jnp.mean(x, axis=-1, keepdims=True)
            x = x * lax.rsqrt(jnp.mean(x * x, axis=-1, keepdims=True) + 1e-5)
            a += [x[:, :HD], x[:, HD:]]
        for n, v in enumerate(_lhs7(*a)):
            xn[n, pl.ds(pl.multiple_of(i * 64, 64), 64), :] = v
        return c
    for i in range(2):
        x_in[i].wait()
        w_in[0][1 + i].start()
        lax.fori_loop(2 * i, 2 * i + 2, first_norm, 0)

    def head_setup(it):
        for m in range(2):
            for i in range(2):
                pl.when(it == i)(w_in[i][m].wait)
            if m == 1:
                @pl.when(it == 0)
                def _():
                    for cp in w_in[1]:
                        cp.start()
            t = qvk_st[m][it, 0:D, 0:256].T
            for i, b in enumerate(_rhs7(t[:128, :HD], t[128:, :HD], t[:128, HD:], t[128:, HD:])):
                wqvt[0][it, i, _tile(m), :] = b
        for i in range(2):
            pl.when(it == i)(w_in[i][2].wait)

        @pl.when(it == 0)
        def _():
            for cp in late_in:
                cp.start()

        for r in range(32):
            prep_keys(None, it, 0, r, None)

    def prep_keys(z, it, e, r, go):
        if go is not None:
            qvk_st[2][z[0] + it, D:D + 8, 0:128] = go.astype(BF)
        blocks = [qvk_st[2][it, k + 16 * r:k + 16 * r + 16, _tile(2 * e + c)] for k in (0, HD) for c in range(2)]
        for n, b in enumerate(_rhs7(*blocks)):
            wk[e][it, n, 16 * (r % 16):16 * (r % 16) + 16, _tile(r // 16)] = b
        return None if go is None else wk_u[e][z[2] + it, 0, 0:8, 0:128]

    def prep_flip(z, it, i, go):
        m, k = divmod(i, NG)
        qvk_st[m][z[0] + it, D:D + 8, 0:128] = go.astype(BF)
        flip[z[0, m], 0:256, _tile(k)] = qvk_st[m][it, _tile(k), 256:512].T
        return flip_u[z[2, m], 0:8, _tile(k)]

    def prep_queries_values(z, it, i, go):
        flip_u[z[0], 128:136, 0:128] = pltpu.bitcast(go, U32)
        r, k = divmod(i, 4)
        m, o = divmod(16 * r, 128)
        blocks = [flip[z[1, m], o + c:o + c + 16, _tile(k + half)] for half in (0, 4) for c in (0, 128)]
        for n, b in enumerate(_rhs7(*blocks)):
            wqvt[1][z[3] + it, n, 16 * r:16 * r + 16, _tile(k)] = b
        return wqvt_u[1][z[2] + it, 0, 0:8, 0:128]

    def prep_out(z, n, r, go):
        src = 256 * (r // 8) + 16 * (r % 8)
        if go is not None:
            wo_st[D:D + 8, 0:128] = go.astype(BF)
            src = pl.multiple_of(z[1], 16) + src
        blocks = [wo_st[pl.ds(src + o, 16), _tile(2 * n + e)] for o in (0, 128) for e in range(2)]
        for m, b in enumerate(_rhs7(*blocks)):
            wo[n][m, 16 * (r % 16):16 * (r % 16) + 16, _tile(r // 16)] = b
        return None if go is None else wo_u[n][z[2], 0:8, 0:128]

    def late_setup():
        for cp in late_in:
            cp.wait()
        for n in range(2):
            for r in range(32):
                prep_out(None, n, r, None)

    lane = lax.broadcasted_iota(I32, (8, 128), 1)

    def prep_spread(z, s, it, i, go):
        perm[0][z[1], 256:264, :] = pltpu.bitcast(go, U32)
        g, k = divmod(i, 4)
        rows = pl.ds(pl.multiple_of(256 * it, 256) + (k >> 1) * HD + (k & 1) * 128, 128)
        w = pltpu.bitcast(wqkv_st[(s - 1) & 3, rows, _tile(g)], U32)
        src = 32 * (lane & 3) + 4 * (((lane >> 4) - g) & 7) + ((lane & 15) >> 2)
        perm[0][z[0, g], 64 * k:64 * k + 64, :] = jnp.take_along_axis(w, _cat([src] * 8, 0), axis=1)
        return perm[0][z[2, g], 64 * k:64 * k + 8, :]

    def prep_exchange(z, i, go):
        perm[0][z[0], 256:264, :] = pltpu.bitcast(go, U32)
        u = [perm[0][z[1, (-j) % NG], 8 * i:8 * i + 8, :] for j in range(NG)]
        for bit in (1, 2, 4):
            m = (lane & (16 * bit)) != 0
            u = [jnp.where(m, u[(j - bit) % NG], u[j]) for j in range(NG)]
        for j in range(NG):
            perm[1][z[0, j], 8 * i:8 * i + 8, :] = u[j]
        return perm[1][z[2], 8 * i:8 * i + 8, :]

    def prep_collect(z, i, go):
        perm[1][z[0], 256:264, :] = pltpu.bitcast(go, U32)
        j, k = divmod(i, 4)
        src = 16 * (((lane >> 2) + j) & 7) + 4 * (lane >> 5) + (lane & 3)
        w = perm[1][z[1, j], 64 * k:64 * k + 64, :]
        perm[2][z[0, j], 64 * k:64 * k + 64, :] = jnp.take_along_axis(w, _cat([src] * 8, 0), axis=1)
        return perm[2][z[2, j], 64 * k:64 * k + 8, :]

    def prep_combine(z, s, it, i, go):
        perm[2][z[0], 256:264, :] = pltpu.bitcast(go, U32)
        r, p = divmod(i, NP)
        w = [pltpu.bitcast(perm[2][z[1, 2 * p + e], o + 8 * r:o + 8 * r + 8, :], BF)
             for o in (0, 128) for e in range(2)]
        rows = pl.ds(pl.multiple_of(256 * it, 256) + 16 * r, 16)
        for n, b in enumerate(_rhs7(*w)):
            wqkv[s, n, rows, _tile(p)] = b
        return pltpu.bitcast(wqkv[z[2] + s, 0, rows, _tile(p)], U32)

    def prep_wob_rows(z, s, h, go):
        wob_st[D:D + 8, 0:128] = go.astype(BF)
        w = wob_st[32 * h:32 * h + 32, pl.ds(pl.multiple_of(s * 256, 256), 256)].astype(F32)
        for e in range(2):
            wob_rows[z[0, e], 33 * h:33 * h + 32, :] = w[:, _tile(e)]
        return wob_rows[z[2], 0:8, :]

    def prep_wob(z, s, i, go):
        wob_rows[z[0], 33 * H:33 * H + 8, :] = go
        d, e = divmod(i, 2)
        blocks = [wob_rows[z[1, c], pl.ds(33 * 16 * e + dd, 16, stride=33), :]
                  for dd in (d, d + DH // 2) for c in range(2)]
        cols = pl.ds(pl.multiple_of(s * 128, 128), 128)
        for n, b in enumerate(_rhs7(*blocks)):
            wob[n, 16 * i:16 * i + 16, cols] = b
        return wob_u[z[2], 0:8, cols]

    def add_residual(s, r0, n, blocks):
        seg = segment(s)
        for y, o in ((_cat(blocks[:2], 1), 0), (_cat(blocks[2:], 1), 128)):
            for i in range(y.shape[0] // 128):
                view = (slice(r0 + TB * i + o, r0 + TB * i + o + 128), slice(256 * n, 256 * n + 256))
                seg[view] = (seg[view].astype(F32) + y[_tile(i)]).astype(BF)

    upper = lane >= 64

    def project(pc, it, e, between=None):
        z = pc.z

        def keys(o, k):
            kk[e][z[0, o]] = k.astype(BF)
            f = _phi(k)
            part, pieces = None, []
            for r in range(0, TB, 32):
                t = f[r:r + 16] + f[r + 16:r + 32]
                part = t[:8] + t[8:] if part is None else part + (t[:8] + t[8:])
                pieces += [f[r:r + 24], pc.after(part, f[r + 24:r + 32])]
            pk[e][z[0, o]] = _cat(pieces, 0).astype(BF)
            part = jnp.sum(part[:, :128] + part[:, 128:], axis=0, keepdims=True)
            zsum[z[0, 2 * e + o]] = jnp.broadcast_to(part, (8, 128))

        def queries_values(c, o, y):
            q, lanes, g = y[:128], slice(TB * c, TB * c + TB), z[0, o]
            for h in range(4):
                qh = q[32 * h:32 * h + 32] * QSCALE
                if h % 2:
                    qh = _cat([pltpu.roll(qh[:, _tile(i)], 64, 1) for i in range(2)], 1)
                qt[e][g, 32 * h:32 * h + 32, lanes] = qh.astype(BF)
            pqt[e][g, :, lanes] = _phi(q).astype(BF)
            vt[e][g, :, lanes] = y[128:].astype(BF)

        pc.strassen(lambda i: _dot(pc.lhs(xn_u[i]), _cat([wk[e][z[1] + it, i, :, _tile(k)] for k in range(2)], 0)),
                    emit_col=keys, between=between)
        for c in range(2):
            pc.strassen(lambda i: _dot_nt(pc.lhs(wqvt_u[e][z[c] + it, i]), xn[i, _tile(c), :]),
                        emit_col=functools.partial(queries_values, c), between=between)

    def scores(z, g, j, t, sbuf, mx):
        zero = jnp.zeros((32, 128), BF)
        q = [qt[g // 2][z[1 + t, g % 2], 32 * h:32 * h + 32, _tile(j)] for h in range(4)]
        n = 64 if t == j else 128
        rows = slice(128 * t, 128 * t + n)
        s = _dot(kk[g // 2][z[1 + j, g % 2], 128 * (t // 2):128 * (t // 2) + n, _tile(t % 2)],
                 _cat([_cat([q[h] if i == h else zero for i in range(4)], 0) for h in range(4)], 1))
        for h in range(4):
            sh = s[:, _tile(h)]
            if t == j:
                sh = sh + bias[h & 1]
            sbuf[z[0], h, rows, :] = sh
            sh = sh if mx[h] is None else _cat([mx[h], sh], 0)
            mx[h] = jnp.max(sh.reshape(-1, 8, 128), axis=0)
        if t < j:
            return
        q = [pltpu.bitcast(jnp.where(_cat([upper == (h % 2 == 0)] * 2, 0), pltpu.bitcast(q[h], U32),
                                     jnp.zeros((16, 128), U32)), BF) for h in range(4)]
        rows = slice(128 * t + 64, 128 * t + 128)
        s = _dot(kk[g // 2][z[1 + j, g % 2], 128 * (t // 2) + 64:128 * (t // 2) + 128, _tile(t % 2)],
                 _cat([_cat([q[0], q[1], zero, zero], 0), _cat([zero, zero, q[2], q[3]], 0)], 1))
        for h in (0, 2):
            sh = s[:, _tile(h // 2)] + bias[2]
            sbuf[z[0], h, rows, :] = sh
            m = jnp.max(sh.reshape(-1, 8, 128), axis=0)
            mx[h] = jnp.where(upper, jnp.maximum(mx[h], m), mx[h])
            mx[h + 1] = jnp.where(upper, mx[h + 1], jnp.maximum(mx[h + 1], m))
        for h in range(4):
            mx[h] = jnp.broadcast_to(jnp.max(mx[h], axis=0, keepdims=True), (8, 128))

    def attend(pc, g, j, t, sbuf, mx, acc, tot):
        z = pc.z

        def probs(h, r, m):
            p = jnp.exp2(sbuf[z[1], h, r:r + 64, :] - _cat([m] * 8, 0))
            part = p[:32] + p[32:]
            part = part[:16] + part[16:]
            return p, part[:8] + part[8:]
        for h in range(4):
            if t < j:
                hi, part = probs(h, 128 * t + 64, mx[h])
            else:
                if h % 2 == 0:
                    shared = probs(h, 128 * t + 64, jnp.where(upper, mx[h], mx[h + 1]))
                mine = upper == (h % 2 == 0)
                hi, part = jnp.where(_cat([mine] * 8, 0), shared[0], 0.0), jnp.where(mine, shared[1], 0.0)
            tot[h] = part if tot[h] is None else tot[h] + part
            hi = [pc.after(tot[h], hi[0:8]), hi[8:]]
            lo, part = probs(h, 128 * t, mx[h])
            tot[h] = tot[h] + part
            p = _cat([pc.after(tot[h], lo[0:8]), lo[8:]] + hi, 0)
            r = _dot(vt[g // 2][z[1 + j, g % 2], 32 * h:32 * h + 32, _tile(t)], p.astype(BF))
            acc[h] = r if acc[h] is None else acc[h] + r

    def memory_read(z, it, g):
        recall[z[0, g]] = _dot(mem[4 * it + g].astype(BF), pqt[g // 2][z[1, g % 2]])

    def memory_update(z, it, g):
        upd = _dot(vt[g // 2][z[5, g % 2]],
                   _cat([pk[g // 2][z[1, g % 2], _tile(t // 2), _tile(t % 2)] for t in range(4)], 0))
        upd = _cat([upd, zsum[z[1, g]]], 0)
        head = lane >> 5
        keep = _cat([head == r // 4 for r in range(16)] + [head == lax.broadcasted_iota(I32, (8, 128), 0)], 0)
        mem[4 * it + g, 0:136, :] = mem[z[1] + 4 * it + g, 0:136, :] + jnp.where(keep, upd, 0.0)

    def gated(z, it, g, j, acc, tot):
        inv_den = _recip(recall[z[1, g], 128:136, _tile(j)] + 1e-6)
        outs = []
        for h in range(4):
            gt = gate[16 * it + 4 * g + h]
            c_dot = (1.0 - gt) * _recip(jnp.broadcast_to(jnp.sum(tot[h], axis=0, keepdims=True), (8, 128)))
            c_mem = gt * jnp.broadcast_to(inv_den[h:h + 1], (8, 128))
            local = acc[h] * _cat([c_dot] * 4, 0)
            if h % 2:
                local = pltpu.roll(local, 64, 1)
            outs.append(local + recall[z[1, g], 32 * h:32 * h + 32, _tile(j)] * _cat([c_mem] * 4, 0))
        return _cat(outs, 0)

    def heads_step(l, s, it, carry):
        pl.when((l == 0) & (s == 0))(functools.partial(head_setup, it))
        pc = _Pacer(tmp, it)
        z = pc.z
        pc.spread(functools.partial(prep_keys, z, it, 1), 32, 0, 4.5, 1.2)
        pc.spread(functools.partial(prep_flip, z, it), 16, 5, 9, 1.8)
        pc.spread(functools.partial(prep_queries_values, z, it), 64, 10, 25, 1.2)
        pc.spread(functools.partial(prep_spread, z, s, it), 32, 0.8, 4.5, 1.8)
        pc.spread(functools.partial(prep_exchange, z), 32, 7, 11, 1.2)
        pc.spread(functools.partial(prep_collect, z), 32, 14, 18, 1.5)
        pc.spread(functools.partial(prep_combine, z, s, it), 64, 22, 39, 1.2)
        order = ((0, 3), (0, 2), (1, 3), (1, 2), (0, 1), (1, 1), (0, 0), (1, 0))
        items = [(2 * p + e, j) for p in range(2) for e, j in order]
        units = [(n, g, j, t) for n, (g, j) in enumerate(items) for t in range(j + 1)]
        state = [([None] * 4, [None] * 4, [None] * 4) for _ in items]
        last = {n: k for k, (n, *_) in enumerate(units)}
        seen = []

        def consume(n, g, j, t):
            attend(pc, g, j, t, sbufs[n % NSLOT], *state[n])
            if t < j:
                return
            o = gated(z, it, g, j, *state[n][1:])
            me = 2 * (j & 1) + (g & 1)
            seen.append(me)
            if len(seen) < 4:
                tiles[me][z[0]] = o
            for i, (x, y, op) in enumerate(LHS7):
                if me in (x, y) and x in seen and y in seen:
                    a, b = [o if q == me else tiles[q][z[1 + me]] for q in (x, y)]
                    oa[it, i, _tile(j // 2), _tile(g // 2)] = op(a, b).astype(BF).T
            if len(seen) == 4:
                seen.clear()

        def rounds():
            reads = (0, 1, 24, 30)
            done, k, updated = 0, 0, 0
            while done < len(units):
                if k in reads:
                    memory_read(z, it, reads.index(k))
                if k < len(units):
                    n, g, j, t = units[k]
                    scores(z, g, j, t, sbufs[n % NSLOT], state[n][0])
                else:
                    memory_update(z, it, updated)
                    updated += 1
                for _ in range(2 if k >= len(units) - 4 else 1):
                    if done < len(units) and last[units[done][0]] + 2 <= k:
                        consume(*units[done])
                        done += 1
                k += 1
                yield
            for g in range(updated, 4):
                memory_update(z, it, g)

        project(pc, it, 0)
        attention = rounds()
        slots = iter(range(21))

        def between():
            if next(slots) >= 5:
                next(attention)
        project(pc, it, 1, between)
        pc.finish()
        for _ in attention:
            pass
        return carry

    def infini_step(l, s, carry):
        lax.fori_loop(0, 2, functools.partial(heads_step, l, s), 0)
        pl.when((l == 0) & (s == 0))(late_setup)
        pc = _Pacer(tmp, s)
        z = pc.z
        nxt = (s + 1) & (NSEG - 1)
        for i in range(SEG // 8):
            norm_mean(z, nxt, i, None)
        pc.spread(functools.partial(norm_var, z, nxt), SEG // 8, 1.5, 5.95, 0)
        pc.spread(functools.partial(norm_store, z), SEG // 8, 9, 26, 1.3)
        for n in range(2, NP):
            pc.spread(functools.partial(prep_out, z, n), 32, 7 * n - 8, 7 * n - 2.3, 1.2)
        pc.spread(functools.partial(prep_wob_rows, z, s), H, 6, 17, 1.5)
        pc.spread(functools.partial(prep_wob, z, s), DH, 19, 26, 1.2)
        for n in range(NP):
            add_residual(s, 0, n, pc.strassen(lambda i: _dot(
                pc.lhs(_cat([oa_u[0, i], oa_u[1, i]], 1)),
                _cat([wo[n][z[1, i], :, _tile(e)] for e in range(2)], 0))))
        pc.finish()
        return carry

    def window_step(l, s, carry):
        pc = _Pacer(tmp, s)
        z = pc.z
        held = {}

        def taps(ref, j, r, n):
            out = [None] * WIN
            for a in range(WIN // 2):
                slab = ref[z[1, j], pl.ds(HALO + r - 8 - DIL * a, n + 8), :]
                out[a] = slab[8:]
                out[a + 4] = slab[:n]
            return out

        def probs(c, i, go):
            kqs[c][z[0, NG], 0:8, :] = go
            i, step = divmod(i, 4)
            r = (i >> 1) * 8 + (i & 1) * 128
            acc = held.pop(("k", c), [None] * WIN)
            for j in (2 * step, 2 * step + 1):
                q = kqs[c][z[1, NG + j], HALO + r:HALO + r + 8, :]
                for w, k in enumerate(taps(kqs[c], j, r, 8)):
                    acc[w] = q * k if j == 0 else acc[w] + q * k
            if step < 3:
                held["k", c] = acc
                return None
            acc = [a + pltpu.roll(a, 64, 1) for a in acc]
            acc = [a + pltpu.roll(a, 32, 1) for a in acc]
            for w in range(WIN):
                if c == 0 and r < DIL * w:
                    pos = s * SEG + r + lax.broadcasted_iota(I32, (8, 128), 0)
                    acc[w] = jnp.where(pos >= DIL * w, acc[w], MASKED)
            m = _tree(jnp.maximum, acc)
            p = [jnp.exp2(a - m) for a in acc]
            inv = _recip(_tree(jnp.add, p))
            for w in range(WIN):
                pbs[c][z[0, w], r:r + 8, :] = p[w] * inv
            return pbs[c][z[2], r:r + 8, :]

        def values(c, i, go):
            i, step = divmod(i, 5)
            r, e = 16 * (i // 4), i % 4
            if step == 4:
                for n, v in enumerate(_lhs7(*held.pop(("v", c)))):
                    obs[c][z[0, n], r:r + 16, _tile(e)] = v
                return pltpu.bitcast(obs[c][z[2], r:r + 16, _tile(e)], U32)
            vbs[c][z[0, NG], 0:8, :] = go
            o, j = r + 128 * (step >> 1), e + 4 * (step & 1)
            y = None
            for w, v in enumerate(taps(vbs[c], j, o, 16)):
                t = pbs[c][z[1 + e, w], o:o + 16, :] * v
                y = t if y is None else y + t
            held.setdefault(("v", c), []).append(y)
            return pltpu.bitcast(y[0:8], U32) | pltpu.bitcast(y[8:16], U32)

        nxt = (s + 1) & (NSEG - 1)
        pc.spread(functools.partial(norm_mean, z, nxt), SEG // 8, 1, 20, 0)
        pc.spread(functools.partial(norm_var, z, nxt), SEG // 8, 21, 53, 4)
        pc.spread(functools.partial(probs, 0), 4 * TB // 8, 58.36, 106, 6.45)
        pc.spread(functools.partial(values, 0), 5 * TB // 8, 147.21, 165.5, 2.28)
        pc.spread(functools.partial(probs, 1), 4 * TB // 8, 112, 146, 5.5)
        pc.spread(functools.partial(values, 1), 5 * TB // 8, 168, 194.33, 2)
        pc.spread(functools.partial(norm_store, z), SEG // 8, 195.9, 214.54, 1.52)

        def project_window(c, part, p):
            refs = vbs if part == 2 else kqs

            def emit(half, e, y):
                if part == 0:
                    y = y * QSCALE
                j = 2 * p + e
                refs[c][z[0, j + (NG if part == 0 else 0)], HALO + 128 * half:HALO + 128 * half + 128, :] = y
                if part > 0 and c == 0 and half == 1:
                    refs[1][z[0, j], 0:HALO, :] = y[128 - HALO:]
            pc.strassen(lambda i: _dot(pc.lhs(xn_u[i, 64 * c:64 * c + 64, :]), wqkv[part + 1, i, :, _tile(p)]), emit)

        for c, part in ((0, 0), (0, 1), (1, 0), (1, 1), (0, 2), (1, 2)):
            for p in range(NP):
                project_window(c, part, p)
        for c in range(2):
            for n in range(NP):
                add_residual(s, TB * c, n, pc.strassen(
                    lambda i: _dot(pc.lhs(obs_u[c][z[1 + n, i]]), wob[i, :, _tile(n)])))
            pl.when(l == 1)(out_copy(s, c).start)
        pc.finish()
        for refs in (kqs, vbs):
            for j in range(NG):
                refs[0][z[0, j], 0:HALO, :] = refs[1][z[2, j], TB:TB + HALO, :]
        return carry

    def layer_pair(l, carry):
        mem[...] = jnp.zeros(mem.shape, F32)
        lax.fori_loop(0, NSEG, functools.partial(infini_step, l), 0)
        for refs in (kqs, vbs):
            refs[0][0:NG, 0:HALO, :] = jnp.zeros((NG, HALO, 128), F32)
        lax.fori_loop(0, NSEG, functools.partial(window_step, l), 0)
        return carry
    lax.fori_loop(0, 2, layer_pair, 0)
    pltpu.make_async_copy(xio, out_hbm, out_sem).wait()


@jax.jit
def pallas_interleave_layers__memory_aug_infini_attn__sliding_local_dilated__prompt_kernel(
    A_x: jax.Array,
    A_wq: jax.Array,
    A_wk: jax.Array,
    A_wv: jax.Array,
    A_wo: jax.Array,
    A_beta: jax.Array,
    B_x: jax.Array,
    B_wqkv: jax.Array,
    B_wo: jax.Array,
):
    del B_x
    hbm = pl.BlockSpec(memory_space=pl.ANY)
    out = pl.pallas_call(
        _kernel,
        out_shape=jax.ShapeDtypeStruct((S, D), BF),
        in_specs=[hbm] * 8,
        out_specs=hbm,
        scratch_shapes=list(_scratch().values()),
        compiler_params=pltpu.CompilerParams(vmem_limit_bytes=110 * 2 ** 20),
        name="fused_layers",
    )(A_x.reshape(S, D), A_wq, A_wk, A_wv, A_wo, A_beta.reshape(1, H), B_wqkv, B_wo)
    return out.reshape(A_x.shape)
```

```python
import functools
import math

import jax
import jax.numpy as jnp
from jax import lax
from jax.experimental import pallas as pl
from jax.experimental.pallas import tpu as pltpu

BF = jnp.bfloat16
F32 = jnp.float32
U32 = jnp.uint32
I32 = jnp.int32

S = 2048
D = 1024
HD = D // 2
H = 32
DH = 32
SEG = 512
NSEG = S // SEG
NG = D // 128
NP = NG // 2
TB = 256
WIN = 8
DIL = 2
HALO = 16
NSLOT = 6
NSEM = 16
LOG2E = math.log2(math.e)
MASKED = -1e9 * LOG2E
QSCALE = DH ** -0.5 * LOG2E


def _dot(a, b):
    return jnp.dot(a, b, preferred_element_type=F32)


def _dot_nt(a, b):
    return lax.dot_general(a, b, (((1,), (1,)), ((), ())), preferred_element_type=F32)


def _phi(t):
    return jnp.where(t > 0, t + 1.0, jnp.exp(t))


def _recip(x):
    r = pltpu.reciprocal(x, approx=True)
    return r * (2.0 - x * r)


def _cat(xs, axis):
    return xs[0] if len(xs) == 1 else jnp.concatenate(xs, axis=axis)


def _tree(op, xs):
    while len(xs) > 1:
        xs = [op(xs[i], xs[i + 1]) for i in range(0, len(xs), 2)]
    return xs[0]


def _tile(j):
    return slice(128 * j, 128 * j + 128)


def _first(a, b):
    del b
    return a


LHS7 = ((0, 3, jnp.add), (2, 3, jnp.add), (0, 0, _first), (3, 3, _first),
        (0, 1, jnp.add), (2, 0, jnp.subtract), (1, 3, jnp.subtract))


def _lhs7(*a):
    return [op(a[x], a[y]).astype(BF) for x, y, op in LHS7]


def _rhs7(b11, b12, b21, b22):
    f11, f12, f21, f22 = [b.astype(F32) for b in (b11, b12, b21, b22)]
    return [b.astype(BF) for b in (f11 + f22, b11, f12 - f22, f21 - f11, b22, f11 + f12, f21 + f22)]


class _Zeros:
    def __init__(self, step):
        self.cache = {(i, 0): step >> (10 + i) for i in range(6)}

    def __getitem__(self, key):
        key = key if isinstance(key, tuple) else (key, 0)
        if key not in self.cache:
            self.cache[key] = self.cache[key[0], 0] + key[1]
        return self.cache[key]


class _Packed:
    def __init__(self, ref):
        self.ref = ref

    def _words(self, idx):
        idx = idx if isinstance(idx, tuple) else (idx,)
        if len(idx) < len(self.ref.shape) - 1 or idx[-2] == slice(None):
            return idx
        return idx[:-2] + (slice(idx[-2].start // 2, idx[-2].stop // 2), idx[-1])

    def __getitem__(self, idx):
        return pltpu.bitcast(self.ref[self._words(idx)], BF)

    def __setitem__(self, idx, value):
        self.ref[self._words(idx)] = pltpu.bitcast(value, U32)


def _bits(x):
    return x if x.dtype == U32 else pltpu.bitcast(x, U32)


class _Pacer:
    def __init__(self, tmp, step):
        self.tmp = tmp
        self.z = _Zeros(step)
        self.no_bits = jnp.full((8, 128), self.z[0].astype(U32))
        self.plan, self.due = {}, {}
        self.pending, self.ready = [], []
        self.count = 0

    def spread(self, fn, n, first, last, slack):
        for i in range(n):
            t = first + i * (last - first) / (n - 1)
            self.plan.setdefault(int(t), []).append((fn, i, t - int(t), slack and t + slack))

    def product(self, thunk):
        for fn, i, go, when in self.pending:
            done = fn(i, go)
            if when and done is not None:
                self.due.setdefault(int(when), []).append((when - int(when), done))
        self.pending = []
        self.ready += self.due.pop(self.count, [])
        y = thunk()
        for fn, i, frac, when in self.plan.pop(self.count, []):
            r = 8 * int(frac * (y.shape[0] // 8))
            self.pending.append((fn, i, y[r:r + 8], when))
        self.count += 1
        return y

    def after(self, t, x):
        bits = _bits(x) | (_bits(t) & _cat([self.no_bits] * (x.shape[1] // 128), 1))
        return bits if x.dtype == U32 else pltpu.bitcast(bits, x.dtype)

    def lhs(self, words):
        if self.ready:
            n = words.shape[0] // 8
            heads = [words[8 * i:8 * i + 8, 0:128] for i in range(n)]
            for frac, t in self.ready:
                heads[int(frac * n)] = self.after(t, heads[int(frac * n)])
            words = _cat([_cat(heads, 0), words[:, 128:]], 1)
            self.ready = []
        return pltpu.bitcast(words, BF)

    def finish(self):
        assert not self.plan and not self.pending

    def strassen(self, prod, emit=None, emit_col=None, between=None):
        def run(i):
            if between:
                between()
            return self.product(functools.partial(prod, i))
        m3 = run(2)
        rows = slice(0, m3.shape[0])

        def put(i, v):
            self.tmp[i][self.z[0], rows, :] = v

        def get(i, n):
            return self.tmp[i][self.z[n], rows, :]
        put(0, m3)
        put(1, run(0))
        put(2, run(6))
        put(3, run(1))
        m5 = run(4)
        c12 = get(0, 1) + m5
        emit(0, 1, c12) if emit else put(5, c12)
        put(4, (get(1, 1) + get(2, 1)) - m5)
        c22 = ((get(1, 2) - get(3, 2)) + get(0, 2)) + run(5)
        if emit_col:
            emit_col(1, _cat([get(5, 1), c22], 1))
        else:
            emit(1, 1, c22) if emit else put(6, c22)
        m4 = run(3)
        c21, c11 = get(3, 1) + m4, get(4, 1) + m4
        if emit_col:
            return emit_col(0, _cat([c11, c21], 1))
        if emit:
            emit(1, 0, c21)
            emit(0, 0, c11)
            return None
        return c11, get(5, 1), c21, get(6, 1)


def _scratch():
    vm = pltpu.VMEM
    return dict(
        xio=vm((S, D), BF),
        xn_u=vm((7, SEG // 4, HD), U32),
        xc=vm((1, SEG, D), F32),
        mean=vm((1, SEG + 32, 128), F32),
        rstd=vm((1, SEG + 32, 128), F32),
        qvk_st=[vm((2, D + 16, HD), BF)] * 3,
        wo_st=vm((D + 16, D), BF),
        wqkv_st=vm((4, D, D), BF),
        wob_st=vm((D + 16, D), BF),
        perm=[vm((NG, 264, 128), U32)] * 3,
        flip_u=vm((2, 136, D), U32),
        wqvt_u=[vm((2, 7, 128, HD), U32)] * 2,
        wk_u=[vm((2, 7, HD // 4, 256), U32)] * 2,
        wqkv_u=vm((4, 7, HD // 2, HD), U32),
        wob_u=vm((7, HD // 2, HD), U32),
        wob_rows=vm((2, 34 * H, 128), F32),
        oa_u=vm((2, 7, SEG // 4, 256), U32),
        mem=vm((NG, 144, 128), F32),
        gate=vm((H, 8, 128), F32),
        bias=vm((3, 64, 128), F32),
        zsum=vm((4, 8, 128), F32),
        recall=vm((4, 144, SEG), F32),
        kqs=[vm((2 * NG, HALO + TB, 128), F32)] * 2,
        vbs=[vm((NG + 2, HALO + TB, 128), F32)] * 2,
        pbs=[vm((WIN, TB, 128), F32)] * 2,
        obs_u=[vm((7, TB // 4, HD), U32)] * 2,
        sems=pltpu.SemaphoreType.DMA((NSEM,)),
        sbufs=[vm((1, 4, SEG, 128), F32)] * NSLOT,
        tmp=[vm((1, 256, 128), F32)] * 7,
        tiles=[vm((1, 128, 128), F32)] * 4,
        qt_u=[vm((2, 64, SEG), U32)] * 2,
        pqt=[vm((2, 128, SEG), BF)] * 2,
        vt_u=[vm((2, 64, SEG), U32)] * 2,
        kk_u=[vm((2, TB // 2, 256), U32)] * 2,
        pk_u=[vm((2, TB // 2, 256), U32)] * 2,
        wo_u=[vm((7, HD // 4, 256), U32)] * NP,
        beta=vm((1, H), BF),
    )


def _kernel(x_hbm, wq_hbm, wk_hbm, wv_hbm, wo_hbm, beta_hbm, wqkv_hbm, wob_hbm, out_hbm,
            xio, xn_u, xc, mean, rstd, qvk_st, wo_st, wqkv_st, wob_st, perm, flip_u,
            wqvt_u, wk_u, wqkv_u, wob_u, wob_rows, oa_u, mem, gate, bias, zsum, recall,
            kqs, vbs, pbs, obs_u, sems, sbufs, tmp, tiles, qt_u, pqt, vt_u, kk_u, pk_u, wo_u, beta):
    oa, xn, flip, wqkv, wob = [_Packed(r) for r in (oa_u, xn_u, flip_u, wqkv_u, wob_u)]
    wqvt, wk, wo, qt, vt, kk, pk, obs = [
        [_Packed(r) for r in refs] for refs in (wqvt_u, wk_u, wo_u, qt_u, vt_u, kk_u, pk_u, obs_u)]

    def segment(s):
        return xio.at[pl.ds(pl.multiple_of(s * SEG, SEG), SEG)]

    sem_ids = iter(range(NSEM))

    def fetch(src, dst):
        return pltpu.make_async_copy(src, dst, sems.at[next(sem_ids)])

    x_in = [fetch(x_hbm.at[pl.ds(r, n)], xio.at[pl.ds(r, n)]) for r, n in ((0, TB), (TB, TB), (SEG, S - SEG))]
    w_in = [[fetch(src.at[:, pl.ds(HD * i, HD)], dst.at[i, pl.ds(0, D)]) for src, dst in zip((wq_hbm, wv_hbm, wk_hbm), qvk_st)]
            for i in range(2)]
    late_in = [x_in[2], fetch(wo_hbm, wo_st.at[pl.ds(0, D)]), fetch(wob_hbm, wob_st.at[pl.ds(0, D)])]
    late_in += [fetch(wqkv_hbm.at[:, pl.ds(D * i, D)], wqkv_st.at[i]) for i in range(3)]
    beta_in = fetch(beta_hbm, beta)
    out_sem = sems.at[next(sem_ids)]

    def out_copy(s, c):
        rows = pl.ds(pl.multiple_of(s * SEG, SEG) + TB * c, TB)
        return pltpu.make_async_copy(xio.at[rows], out_hbm.at[rows], out_sem)

    def norm_mean(z, s, i, go):
        if go is not None:
            mean[z[1], SEG:SEG + 8, :] = go
        rows = slice(8 * i, 8 * i + 8)
        m = jnp.mean(segment(s)[rows, :].astype(F32), axis=-1, keepdims=True)
        mean[z[0], rows, :] = jnp.broadcast_to(m, (8, 128))

    def norm_var(z, s, i, go):
        mean[z[0], SEG:SEG + 8, :] = go
        rows = slice(8 * i, 8 * i + 8)
        x = segment(s + z[0])[rows, :].astype(F32) - _cat([mean[z[1], rows, :]] * NG, 1)
        xc[z[0], rows, :] = x
        v = jnp.mean(x * x, axis=-1, keepdims=True)
        rstd[z[0], rows, :] = lax.rsqrt(jnp.broadcast_to(v, (8, 128)) + 1e-5)
        return rstd[z[2], rows, :]

    def norm_store(z, i, go):
        rstd[z[0], SEG:SEG + 8, :] = go
        i, e = divmod(i, 4)
        c, r = divmod(16 * i, 128)
        a = [xc[z[1], o:o + 16, _tile(j)] * rstd[z[1], o:o + 16, :]
             for o in (TB * c + r, TB * c + r + 128) for j in (e, 4 + e)]
        for n, v in enumerate(_lhs7(*a)):
            xn[n, 16 * i:16 * i + 16, _tile(e)] = v
        return xn_u[z[2], 8 * i:8 * i + 8, _tile(e)]

    for cp in (beta_in, x_in[0], x_in[1], w_in[0][0]):
        cp.start()

    key = lax.broadcasted_iota(I32, (64, 128), 0)
    col = lax.broadcasted_iota(I32, (64, 128), 1)
    for i, query in enumerate((col, col ^ 64, col & 63)):
        bias[i] = jnp.where(key <= query, 0.0, MASKED)
    beta_in.wait()
    diag = lax.broadcasted_iota(I32, (H, H), 0) == lax.broadcasted_iota(I32, (H, H), 1)
    b_row = jnp.broadcast_to(beta[...].astype(F32), (H, H))
    b_col = jnp.sum(jnp.where(diag, b_row, 0.0), axis=1, keepdims=True)
    g_all = jax.nn.sigmoid(jnp.broadcast_to(b_col, (H, 128)))
    for h in range(H):
        gate[h] = jnp.broadcast_to(g_all[h:h + 1], (8, 128))

    def clear(i, c):
        wqkv_st[3, pl.ds(pl.multiple_of(i * 128, 128), 128), :] = jnp.zeros((128, D), BF)
        return c
    lax.fori_loop(0, D // 128, clear, 0)

    def first_norm(i, c):
        r = (i >> 1) * TB + (i & 1) * 64
        a = []
        for o in (0, 128):
            x = xio[pl.ds(pl.multiple_of(r + o, 64), 64), :].astype(F32)
            x = x - jnp.mean(x, axis=-1, keepdims=True)
            x = x * lax.rsqrt(jnp.mean(x * x, axis=-1, keepdims=True) + 1e-5)
            a += [x[:, :HD], x[:, HD:]]
        for n, v in enumerate(_lhs7(*a)):
            xn_u[n, pl.ds(pl.multiple_of(i * 32, 32), 32), :] = _bits(v)
        return c
    for i in range(2):
        x_in[i].wait()
        w_in[0][1 + i].start()
        lax.fori_loop(2 * i, 2 * i + 2, first_norm, 0)

    def head_setup(it):
        for m in range(2):
            for i in range(2):
                pl.when(it == i)(w_in[i][m].wait)
            if m == 1:
                @pl.when(it == 0)
                def _():
                    for cp in w_in[1]:
                        cp.start()
            t = qvk_st[m][it, 0:D, 0:256].T
            for i, b in enumerate(_rhs7(t[:128, :HD], t[128:, :HD], t[:128, HD:], t[128:, HD:])):
                wqvt[0][it, i, _tile(m), :] = b
        for i in range(2):
            pl.when(it == i)(w_in[i][2].wait)

        @pl.when(it == 0)
        def _():
            for cp in late_in:
                cp.start()

        for r in range(32):
            prep_keys(None, it, 0, r, None)

    def prep_keys(z, it, e, r, go):
        if go is not None:
            qvk_st[2][z[0] + it, D:D + 8, 0:128] = go.astype(BF)
        blocks = [qvk_st[2][it, k + 16 * r:k + 16 * r + 16, _tile(2 * e + c)] for k in (0, HD) for c in range(2)]
        for n, b in enumerate(_rhs7(*blocks)):
            wk[e][it, n, 16 * (r % 16):16 * (r % 16) + 16, _tile(r // 16)] = b
        return None if go is None else wk_u[e][z[2] + it, 0, 0:8, 0:128]

    def prep_flip(z, it, i, go):
        m, k = divmod(i, NG)
        qvk_st[m][z[0] + it, D:D + 8, 0:128] = go.astype(BF)
        flip[z[0, m], 0:256, _tile(k)] = qvk_st[m][it, _tile(k), 256:512].T
        return flip_u[z[2, m], 0:8, _tile(k)]

    def prep_queries_values(z, it, i, go):
        flip_u[z[0], 128:136, 0:128] = pltpu.bitcast(go, U32)
        r, k = divmod(i, 4)
        m, o = divmod(16 * r, 128)
        blocks = [flip[z[1, m], o + c:o + c + 16, _tile(k + half)] for half in (0, 4) for c in (0, 128)]
        for n, b in enumerate(_rhs7(*blocks)):
            wqvt[1][z[3] + it, n, 16 * r:16 * r + 16, _tile(k)] = b
        return wqvt_u[1][z[2] + it, 0, 0:8, 0:128]

    def prep_out(z, n, r, go):
        src = 256 * (r // 8) + 16 * (r % 8)
        if go is not None:
            wo_st[D:D + 8, 0:128] = go.astype(BF)
            src = pl.multiple_of(z[1], 16) + src
        blocks = [wo_st[pl.ds(src + o, 16), _tile(2 * n + e)] for o in (0, 128) for e in range(2)]
        for m, b in enumerate(_rhs7(*blocks)):
            wo[n][m, 16 * (r % 16):16 * (r % 16) + 16, _tile(r // 16)] = b
        return None if go is None else wo_u[n][z[2], 0:8, 0:128]

    def late_setup():
        for cp in late_in:
            cp.wait()
        for n in range(2):
            for r in range(32):
                prep_out(None, n, r, None)

    lane = lax.broadcasted_iota(I32, (8, 128), 1)

    def prep_spread(z, s, it, i, go):
        perm[0][z[1], 256:264, :] = pltpu.bitcast(go, U32)
        g, k = divmod(i, 4)
        rows = pl.ds(pl.multiple_of(256 * it, 256) + (k >> 1) * HD + (k & 1) * 128, 128)
        w = pltpu.bitcast(wqkv_st[(s - 1) & 3, rows, _tile(g)], U32)
        src = 32 * (lane & 3) + 4 * (((lane >> 4) - g) & 7) + ((lane & 15) >> 2)
        perm[0][z[0, g], 64 * k:64 * k + 64, :] = jnp.take_along_axis(w, _cat([src] * 8, 0), axis=1)
        return perm[0][z[2, g], 64 * k:64 * k + 8, :]

    def prep_exchange(z, i, go):
        perm[0][z[0], 256:264, :] = pltpu.bitcast(go, U32)
        u = [perm[0][z[1, (-j) % NG], 8 * i:8 * i + 8, :] for j in range(NG)]
        for bit in (1, 2, 4):
            m = (lane & (16 * bit)) != 0
            u = [jnp.where(m, u[(j - bit) % NG], u[j]) for j in range(NG)]
        for j in range(NG):
            perm[1][z[0, j], 8 * i:8 * i + 8, :] = u[j]
        return perm[1][z[2], 8 * i:8 * i + 8, :]

    def prep_collect(z, i, go):
        perm[1][z[0], 256:264, :] = pltpu.bitcast(go, U32)
        j, k = divmod(i, 4)
        src = 16 * (((lane >> 2) + j) & 7) + 4 * (lane >> 5) + (lane & 3)
        w = perm[1][z[1, j], 64 * k:64 * k + 64, :]
        perm[2][z[0, j], 64 * k:64 * k + 64, :] = jnp.take_along_axis(w, _cat([src] * 8, 0), axis=1)
        return perm[2][z[2, j], 64 * k:64 * k + 8, :]

    def prep_combine(z, s, it, i, go):
        perm[2][z[0], 256:264, :] = pltpu.bitcast(go, U32)
        r, p = divmod(i, NP)
        w = [pltpu.bitcast(perm[2][z[1, 2 * p + e], o + 8 * r:o + 8 * r + 8, :], BF)
             for o in (0, 128) for e in range(2)]
        rows = pl.ds(pl.multiple_of(128 * it, 128) + 8 * r, 8)
        for n, b in enumerate(_rhs7(*w)):
            wqkv_u[s, n, rows, _tile(p)] = _bits(b)
        return wqkv_u[z[2] + s, 0, rows, _tile(p)]

    def prep_wob_rows(z, s, h, go):
        wob_st[D:D + 8, 0:128] = go.astype(BF)
        w = wob_st[32 * h:32 * h + 32, pl.ds(pl.multiple_of(s * 256, 256), 256)].astype(F32)
        for e in range(2):
            wob_rows[z[0, e], 33 * h:33 * h + 32, :] = w[:, _tile(e)]
        return wob_rows[z[2], 0:8, :]

    def prep_wob(z, s, i, go):
        wob_rows[z[0], 33 * H:33 * H + 8, :] = go
        d, e = divmod(i, 2)
        blocks = [wob_rows[z[1, c], pl.ds(33 * 16 * e + dd, 16, stride=33), :]
                  for dd in (d, d + DH // 2) for c in range(2)]
        cols = pl.ds(pl.multiple_of(s * 128, 128), 128)
        for n, b in enumerate(_rhs7(*blocks)):
            wob[n, 16 * i:16 * i + 16, cols] = b
        return wob_u[z[2], 0:8, cols]

    def add_residual(s, r0, n, blocks):
        seg = segment(s)
        for y, o in ((_cat(blocks[:2], 1), 0), (_cat(blocks[2:], 1), 128)):
            for i in range(y.shape[0] // 128):
                view = (slice(r0 + TB * i + o, r0 + TB * i + o + 128), slice(256 * n, 256 * n + 256))
                seg[view] = (seg[view].astype(F32) + y[_tile(i)]).astype(BF)

    upper = lane >= 64

    def project(pc, it, e, between=None):
        z = pc.z

        def keys(o, k):
            kk[e][z[0, o]] = k.astype(BF)
            f = _phi(k)
            part, pieces = None, []
            for r in range(0, TB, 32):
                t = f[r:r + 16] + f[r + 16:r + 32]
                part = t[:8] + t[8:] if part is None else part + (t[:8] + t[8:])
                pieces += [f[r:r + 24], pc.after(part, f[r + 24:r + 32])]
            pk[e][z[0, o]] = _cat(pieces, 0).astype(BF)
            part = jnp.sum(part[:, :128] + part[:, 128:], axis=0, keepdims=True)
            zsum[z[0, 2 * e + o]] = jnp.broadcast_to(part, (8, 128))

        def queries_values(c, o, y):
            q, lanes, g = y[:128], slice(TB * c, TB * c + TB), z[0, o]
            for h in range(4):
                qh = q[32 * h:32 * h + 32] * QSCALE
                if h % 2:
                    qh = _cat([pltpu.roll(qh[:, _tile(i)], 64, 1) for i in range(2)], 1)
                qt[e][g, 32 * h:32 * h + 32, lanes] = qh.astype(BF)
            pqt[e][g, :, lanes] = _phi(q).astype(BF)
            vt[e][g, :, lanes] = y[128:].astype(BF)

        pc.strassen(lambda i: _dot(pc.lhs(xn_u[i]), _cat([wk[e][z[1] + it, i, :, _tile(k)] for k in range(2)], 0)),
                    emit_col=keys, between=between)
        for c in range(2):
            pc.strassen(lambda i: _dot_nt(pc.lhs(wqvt_u[e][z[c] + it, i]), xn[i, _tile(c), :]),
                        emit_col=functools.partial(queries_values, c), between=between)

    def scores(z, g, j, t, sbuf, mx):
        zero = jnp.zeros((32, 128), BF)
        q = [qt[g // 2][z[1 + t, g % 2], 32 * h:32 * h + 32, _tile(j)] for h in range(4)]
        n = 64 if t == j else 128
        rows = slice(128 * t, 128 * t + n)
        s = _dot(kk[g // 2][z[1 + j, g % 2], 128 * (t // 2):128 * (t // 2) + n, _tile(t % 2)],
                 _cat([_cat([q[h] if i == h else zero for i in range(4)], 0) for h in range(4)], 1))
        for h in range(4):
            sh = s[:, _tile(h)]
            if t == j:
                sh = sh + bias[h & 1]
            sbuf[z[0], h, rows, :] = sh
            sh = sh if mx[h] is None else _cat([mx[h], sh], 0)
            mx[h] = jnp.max(sh.reshape(-1, 8, 128), axis=0)
        if t < j:
            return
        q = [pltpu.bitcast(jnp.where(_cat([upper == (h % 2 == 0)] * 2, 0), pltpu.bitcast(q[h], U32),
                                     jnp.zeros((16, 128), U32)), BF) for h in range(4)]
        rows = slice(128 * t + 64, 128 * t + 128)
        s = _dot(kk[g // 2][z[1 + j, g % 2], 128 * (t // 2) + 64:128 * (t // 2) + 128, _tile(t % 2)],
                 _cat([_cat([q[0], q[1], zero, zero], 0), _cat([zero, zero, q[2], q[3]], 0)], 1))
        for h in (0, 2):
            sh = s[:, _tile(h // 2)] + bias[2]
            sbuf[z[0], h, rows, :] = sh
            m = jnp.max(sh.reshape(-1, 8, 128), axis=0)
            mx[h] = jnp.where(upper, jnp.maximum(mx[h], m), mx[h])
            mx[h + 1] = jnp.where(upper, mx[h + 1], jnp.maximum(mx[h + 1], m))
        for h in range(4):
            mx[h] = jnp.broadcast_to(jnp.max(mx[h], axis=0, keepdims=True), (8, 128))

    def attend(pc, g, j, t, sbuf, mx, acc, tot):
        z = pc.z

        def probs(h, r, m):
            p = jnp.exp2(sbuf[z[1], h, r:r + 64, :] - _cat([m] * 8, 0))
            part = p[:32] + p[32:]
            part = part[:16] + part[16:]
            return p, part[:8] + part[8:]
        for h in range(4):
            if t < j:
                hi, part = probs(h, 128 * t + 64, mx[h])
            else:
                if h % 2 == 0:
                    shared = probs(h, 128 * t + 64, jnp.where(upper, mx[h], mx[h + 1]))
                mine = upper == (h % 2 == 0)
                hi, part = jnp.where(_cat([mine] * 8, 0), shared[0], 0.0), jnp.where(mine, shared[1], 0.0)
            tot[h] = part if tot[h] is None else tot[h] + part
            hi = [pc.after(tot[h], hi[0:8]), hi[8:]]
            lo, part = probs(h, 128 * t, mx[h])
            tot[h] = tot[h] + part
            p = _cat([pc.after(tot[h], lo[0:8]), lo[8:]] + hi, 0)
            r = _dot(vt[g // 2][z[1 + j, g % 2], 32 * h:32 * h + 32, _tile(t)], p.astype(BF))
            acc[h] = r if acc[h] is None else acc[h] + r

    def memory_read(z, it, g):
        recall[z[0, g]] = _dot(mem[4 * it + g].astype(BF), pqt[g // 2][z[1, g % 2]])

    def memory_update(z, it, g):
        upd = _dot(vt[g // 2][z[5, g % 2]],
                   _cat([pk[g // 2][z[1, g % 2], _tile(t // 2), _tile(t % 2)] for t in range(4)], 0))
        upd = _cat([upd, zsum[z[1, g]]], 0)
        head = lane >> 5
        keep = _cat([head == r // 4 for r in range(16)] + [head == lax.broadcasted_iota(I32, (8, 128), 0)], 0)
        mem[4 * it + g, 0:136, :] = mem[z[1] + 4 * it + g, 0:136, :] + jnp.where(keep, upd, 0.0)

    def gated(z, it, g, j, acc, tot):
        inv_den = _recip(recall[z[1, g], 128:136, _tile(j)] + 1e-6)
        outs = []
        for h in range(4):
            gt = gate[16 * it + 4 * g + h]
            c_dot = (1.0 - gt) * _recip(jnp.broadcast_to(jnp.sum(tot[h], axis=0, keepdims=True), (8, 128)))
            c_mem = gt * jnp.broadcast_to(inv_den[h:h + 1], (8, 128))
            local = acc[h] * _cat([c_dot] * 4, 0)
            if h % 2:
                local = pltpu.roll(local, 64, 1)
            outs.append(local + recall[z[1, g], 32 * h:32 * h + 32, _tile(j)] * _cat([c_mem] * 4, 0))
        return _cat(outs, 0)

    def heads_step(l, s, it, carry):
        pl.when((l == 0) & (s == 0))(functools.partial(head_setup, it))
        pc = _Pacer(tmp, it)
        z = pc.z
        pc.spread(functools.partial(prep_keys, z, it, 1), 32, 0, 4.5, 1.2)
        pc.spread(functools.partial(prep_flip, z, it), 16, 5, 9, 1.8)
        pc.spread(functools.partial(prep_queries_values, z, it), 64, 10, 25, 1.2)
        pc.spread(functools.partial(prep_spread, z, s, it), 32, 0.8, 4.5, 1.8)
        pc.spread(functools.partial(prep_exchange, z), 32, 7, 11, 1.2)
        pc.spread(functools.partial(prep_collect, z), 32, 14, 18, 1.5)
        pc.spread(functools.partial(prep_combine, z, s, it), 64, 22, 39, 1.2)
        order = ((0, 3), (0, 2), (1, 3), (1, 2), (0, 1), (1, 1), (0, 0), (1, 0))
        items = [(2 * p + e, j) for p in range(2) for e, j in order]
        units = [(n, g, j, t) for n, (g, j) in enumerate(items) for t in range(j + 1)]
        state = [([None] * 4, [None] * 4, [None] * 4) for _ in items]
        last = {n: k for k, (n, *_) in enumerate(units)}
        seen = []

        def consume(n, g, j, t):
            attend(pc, g, j, t, sbufs[n % NSLOT], *state[n])
            if t < j:
                return
            o = gated(z, it, g, j, *state[n][1:])
            me = 2 * (j & 1) + (g & 1)
            seen.append(me)
            if len(seen) < 4:
                tiles[me][z[0]] = o
            for i, (x, y, op) in enumerate(LHS7):
                if me in (x, y) and x in seen and y in seen:
                    a, b = [o if q == me else tiles[q][z[1 + me]] for q in (x, y)]
                    oa[it, i, _tile(j // 2), _tile(g // 2)] = op(a, b).astype(BF).T
            if len(seen) == 4:
                seen.clear()

        def rounds():
            reads = (0, 1, 24, 30)
            done, k, updated = 0, 0, 0
            while done < len(units):
                if k in reads:
                    memory_read(z, it, reads.index(k))
                if k < len(units):
                    n, g, j, t = units[k]
                    scores(z, g, j, t, sbufs[n % NSLOT], state[n][0])
                else:
                    memory_update(z, it, updated)
                    updated += 1
                for _ in range(2 if k >= len(units) - 4 else 1):
                    if done < len(units) and last[units[done][0]] + 2 <= k:
                        consume(*units[done])
                        done += 1
                k += 1
                yield
            for g in range(updated, 4):
                memory_update(z, it, g)

        project(pc, it, 0)
        attention = rounds()
        slots = iter(range(21))

        def between():
            if next(slots) >= 5:
                next(attention)
        project(pc, it, 1, between)
        pc.finish()
        for _ in attention:
            pass
        return carry

    def infini_step(l, s, carry):
        lax.fori_loop(0, 2, functools.partial(heads_step, l, s), 0)
        pl.when((l == 0) & (s == 0))(late_setup)
        pc = _Pacer(tmp, s)
        z = pc.z
        nxt = (s + 1) & (NSEG - 1)
        for i in range(SEG // 8):
            norm_mean(z, nxt, i, None)
        pc.spread(functools.partial(norm_var, z, nxt), SEG // 8, 1.5, 5.95, 0)
        pc.spread(functools.partial(norm_store, z), SEG // 8, 9, 26, 1.3)
        for n in range(2, NP):
            pc.spread(functools.partial(prep_out, z, n), 32, 7 * n - 8, 7 * n - 2.3, 1.2)
        pc.spread(functools.partial(prep_wob_rows, z, s), H, 6, 17, 1.5)
        pc.spread(functools.partial(prep_wob, z, s), DH, 19, 26, 1.2)
        for n in range(NP):
            add_residual(s, 0, n, pc.strassen(lambda i: _dot(
                pc.lhs(_cat([oa_u[0, i], oa_u[1, i]], 1)),
                _cat([wo[n][z[1, i], :, _tile(e)] for e in range(2)], 0))))
        pc.finish()
        return carry

    def window_step(l, s, carry):
        pc = _Pacer(tmp, s)
        z = pc.z
        held = {}

        def taps(ref, j, r, n):
            out = [None] * WIN
            for a in range(WIN // 2):
                slab = ref[z[1, j], pl.ds(HALO + r - 8 - DIL * a, n + 8), :]
                out[a] = slab[8:]
                out[a + 4] = slab[:n]
            return out

        def probs(c, i, go):
            kqs[c][z[0, NG], 0:8, :] = go
            i, step = divmod(i, 4)
            r = (i >> 1) * 8 + (i & 1) * 128
            acc = held.pop(("k", c), [None] * WIN)
            for j in (2 * step, 2 * step + 1):
                q = kqs[c][z[1, NG + j], HALO + r:HALO + r + 8, :]
                for w, k in enumerate(taps(kqs[c], j, r, 8)):
                    acc[w] = q * k if j == 0 else acc[w] + q * k
            if step < 3:
                held["k", c] = acc
                return None
            acc = [a + pltpu.roll(a, 64, 1) for a in acc]
            acc = [a + pltpu.roll(a, 32, 1) for a in acc]
            for w in range(WIN):
                if c == 0 and r < DIL * w:
                    pos = s * SEG + r + lax.broadcasted_iota(I32, (8, 128), 0)
                    acc[w] = jnp.where(pos >= DIL * w, acc[w], MASKED)
            m = _tree(jnp.maximum, acc)
            p = [jnp.exp2(a - m) for a in acc]
            inv = _recip(_tree(jnp.add, p))
            for w in range(WIN):
                pbs[c][z[0, w], r:r + 8, :] = p[w] * inv
            return pbs[c][z[2], r:r + 8, :]

        def values(c, i, go):
            i, step = divmod(i, 5)
            r, e = 16 * (i // 4), i % 4
            if step == 4:
                for n, v in enumerate(_lhs7(*held.pop(("v", c)))):
                    obs[c][z[0, n], r:r + 16, _tile(e)] = v
                return obs_u[c][z[2], r // 2:r // 2 + 8, _tile(e)]
            vbs[c][z[0, NG], 0:8, :] = go
            o, j = r + 128 * (step >> 1), e + 4 * (step & 1)
            y = None
            for w, v in enumerate(taps(vbs[c], j, o, 16)):
                t = pbs[c][z[1 + e, w], o:o + 16, :] * v
                y = t if y is None else y + t
            held.setdefault(("v", c), []).append(y)
            return pltpu.bitcast(y[0:8], U32) | pltpu.bitcast(y[8:16], U32)

        nxt = (s + 1) & (NSEG - 1)
        pc.spread(functools.partial(norm_mean, z, nxt), SEG // 8, 1, 20, 0)
        pc.spread(functools.partial(norm_var, z, nxt), SEG // 8, 21, 53, 4)
        pc.spread(functools.partial(probs, 0), 4 * TB // 8, 58.36, 106, 6.45)
        pc.spread(functools.partial(values, 0), 5 * TB // 8, 147.21, 165.5, 2.28)
        pc.spread(functools.partial(probs, 1), 4 * TB // 8, 112, 146, 5.5)
        pc.spread(functools.partial(values, 1), 5 * TB // 8, 168, 194.33, 2)
        pc.spread(functools.partial(norm_store, z), SEG // 8, 195.9, 214.54, 1.52)

        def project_window(c, part, p):
            refs = vbs if part == 2 else kqs

            def emit(half, e, y):
                if part == 0:
                    y = y * QSCALE
                j = 2 * p + e
                refs[c][z[0, j + (NG if part == 0 else 0)], HALO + 128 * half:HALO + 128 * half + 128, :] = y
                if part > 0 and c == 0 and half == 1:
                    refs[1][z[0, j], 0:HALO, :] = y[128 - HALO:]
            pc.strassen(lambda i: _dot(pc.lhs(xn_u[i, 64 * c:64 * c + 64, :]), wqkv[part + 1, i, :, _tile(p)]), emit)

        for c, part in ((0, 0), (0, 1), (1, 0), (1, 1), (0, 2), (1, 2)):
            for p in range(NP):
                project_window(c, part, p)
        for c in range(2):
            for n in range(NP):
                add_residual(s, TB * c, n, pc.strassen(
                    lambda i: _dot(pc.lhs(obs_u[c][z[1 + n, i]]), wob[i, :, _tile(n)])))
            pl.when(l == 1)(out_copy(s, c).start)
        pc.finish()
        for refs in (kqs, vbs):
            for j in range(NG):
                refs[0][z[0, j], 0:HALO, :] = refs[1][z[2, j], TB:TB + HALO, :]
        return carry

    def layer_pair(l, carry):
        mem[...] = jnp.zeros(mem.shape, F32)
        lax.fori_loop(0, NSEG, functools.partial(infini_step, l), 0)
        for refs in (kqs, vbs):
            refs[0][0:NG, 0:HALO, :] = jnp.zeros((NG, HALO, 128), F32)
        lax.fori_loop(0, NSEG, functools.partial(window_step, l), 0)
        return carry
    lax.fori_loop(0, 2, layer_pair, 0)
    pltpu.make_async_copy(xio, out_hbm, out_sem).wait()


@jax.jit
def pallas_interleave_layers__memory_aug_infini_attn__sliding_local_dilated__prompt_kernel(
    A_x: jax.Array,
    A_wq: jax.Array,
    A_wk: jax.Array,
    A_wv: jax.Array,
    A_wo: jax.Array,
    A_beta: jax.Array,
    B_x: jax.Array,
    B_wqkv: jax.Array,
    B_wo: jax.Array,
):
    del B_x
    hbm = pl.BlockSpec(memory_space=pl.ANY)
    out = pl.pallas_call(
        _kernel,
        out_shape=jax.ShapeDtypeStruct((S, D), BF),
        in_specs=[hbm] * 8,
        out_specs=hbm,
        scratch_shapes=list(_scratch().values()),
        compiler_params=pltpu.CompilerParams(vmem_limit_bytes=110 * 2 ** 20),
        name="fused_layers",
    )(A_x.reshape(S, D), A_wq, A_wk, A_wv, A_wo, A_beta.reshape(1, H), B_wqkv, B_wo)
    return out.reshape(A_x.shape)
```
